```python
import jax
import jax.numpy as jnp

def _softmax(x, axis=-1):
    return jax.nn.softmax(x, axis=axis)

def _gelu(x):
    return jax.nn.gelu(x, approximate=True)

def _silu(x):
    return jax.nn.silu(x)

def _sigmoid(x):
    return jax.nn.sigmoid(x)

def _layernorm(x, axis=-1, eps=1e-05):
    m = jnp.mean(x, axis=axis, keepdims=True)
    v = jnp.var(x, axis=axis, keepdims=True)
    return (x - m) / jnp.sqrt(v + eps)

def _scatter_add(tgt, idx, src, axis=0):
    return tgt.at[idx].add(src)

def _segment_sum(src, seg, n):
    return jax.ops.segment_sum(src, seg, n)

class _Rng:

    def __init__(self, key):
        self._k = key

    def _next(self):
        self._k, sub = jax.random.split(self._k)
        return sub

    def normal(self, shape):
        return jax.random.normal(self._next(), shape, dtype=jnp.bfloat16)

    def randint(self, lo, hi, shape):
        return jax.random.randint(self._next(), shape, lo, hi, dtype=jnp.int32)

    def uniform(self, shape, lo=0.0, hi=1.0):
        return jax.random.uniform(self._next(), shape, jnp.bfloat16, lo, hi)

    def permutation(self, n):
        return jax.random.permutation(self._next(), n)
kernel_name = 'adaLN_cond__sliding_block_cached__moe_arch_mod__decode'

def setup_inputs():
    _rng = _Rng(jax.random.key(int.from_bytes(__import__("os").urandom(4), "little")))
    _w = lambda a: (lambda t: t.astype(jnp.bfloat16) if jnp.issubdtype(t.dtype, jnp.floating) else t)(jnp.asarray(a))

    def _A_setup():
        B, Sq, D = (8, 1, 576)
        Hq, Hkv, Sk, Dh = (32, 16, 8192, 128)
        assert Hq % Hkv == 0, (Hq, Hkv)
        return {'x': _w((lambda *s: _rng.normal(s) * 0.05)(B, Sq, D)), 'k_cache': _w((lambda *s: _rng.normal(s) * 0.05)(B, Hkv, Sk, Dh)), 'v_cache': _w((lambda *s: _rng.normal(s) * 0.05)(B, Hkv, Sk, Dh)), 'wq': _w((lambda *s: _rng.normal(s) * 0.05)(D, Hq * Dh) * D ** (-0.5)), 'wo': _w((lambda *s: _rng.normal(s) * 0.05)(Hq * Dh, D) * (Hq * Dh) ** (-0.5))}
    _A_in = _A_setup()

    def _B_setup():
        B, S, D, F, C = (8, 1, 576, 4608, 1)
        return {'x': _w((lambda *s: _rng.normal(s) * 0.05)(B, S, D)), 'w_r': _w((lambda *s: _rng.normal(s) * 0.05)(D)), 'w_gate': _w((lambda *s: _rng.normal(s) * 0.05)(D, F)), 'w_up': _w((lambda *s: _rng.normal(s) * 0.05)(D, F)), 'w_down': _w((lambda *s: _rng.normal(s) * 0.05)(F, D))}
    _B_in = _B_setup()
    return {'A_x': _A_in['x'], 'A_k_cache': _A_in['k_cache'], 'A_v_cache': _A_in['v_cache'], 'A_wq': _A_in['wq'], 'A_wo': _A_in['wo'], 'B_x': _B_in['x'], 'B_w_r': _B_in['w_r'], 'B_w_gate': _B_in['w_gate'], 'B_w_up': _B_in['w_up'], 'B_w_down': _B_in['w_down'], 'c': _w((lambda *s: _rng.normal(s) * 0.05)(8, 576)), 'w_mod': _w((lambda *s: _rng.normal(s) * 0.05)(576, 6 * 576) * 576 ** (-0.5))}

def reference(A_x, A_k_cache, A_v_cache, A_wq, A_wo, B_x, B_w_r, B_w_gate, B_w_up, B_w_down, c, w_mod):

    def _A_ref(x, k_cache, v_cache, wq, wo):
        B, Sq, D = x.shape
        Hq, Dh = (32, 128)
        Hkv, Sk = (k_cache.shape[1], k_cache.shape[2])
        W = min(4096, max(256, Sk // 4))
        rep = Hq // Hkv
        q = (lambda x, *d: x.transpose(*d))((x @ wq).reshape(B, Sq, Hq, Dh), 0, 2, 1, 3)
        k = jnp.repeat(k_cache[:, :, Sk - W:, :], rep, axis=1)
        v = jnp.repeat(v_cache[:, :, Sk - W:, :], rep, axis=1)
        scores = jnp.einsum('bhqd,bhkd->bhqk', q, k) * Dh ** (-0.5)
        p = _softmax(scores, axis=-1)
        o = jnp.einsum('bhqk,bhkd->bhqd', p, v)
        return (lambda x, *d: x.transpose(*d))(o, 0, 2, 1, 3).reshape(B, Sq, Hq * Dh) @ wo

    def _B_ref(x, w_r, w_gate, w_up, w_down):
        B, S, D = x.shape
        C = 1
        r = x @ w_r
        idx = jnp.argsort(-r, axis=-1)[:, :C]
        idx_e = jnp.repeat(idx.reshape(B, C, 1), D, axis=2)
        x_sel = jnp.take_along_axis(x, idx_e, axis=1)
        g = _silu(x_sel @ w_gate)
        u = x_sel @ w_up
        y = g * u @ w_down
        r_sel = _sigmoid(jnp.take_along_axis(r, idx, axis=1))
        y = y * r_sel.reshape(B, C, 1)
        b_off = (jnp.arange(B) * S).reshape(B, 1)
        flat_idx = (idx + b_off).reshape(B * C)
        zero = (x * 0.0).reshape(B * S, D)
        upd = _scatter_add(zero, flat_idx, y.reshape(B * C, D), axis=0)
        return x + upd.reshape(B, S, D)
    x = A_x
    mod = (_silu(c) @ w_mod).reshape(c.shape[0], 6, 1, -1)
    sa, ca, ga, sb, cb, gb = (mod[:, 0].copy(), mod[:, 1].copy(), mod[:, 2].copy(), mod[:, 3].copy(), mod[:, 4].copy(), mod[:, 5].copy())
    h = _layernorm(x, axis=-1) * (1 + ca) + sa
    x = x + ga * _A_ref(h, A_k_cache, A_v_cache, A_wq, A_wo)
    h = _layernorm(x, axis=-1) * (1 + cb) + sb
    x = x + gb * _B_ref(h, B_w_r, B_w_gate, B_w_up, B_w_down)
    return x
```

```python
import functools

import jax
import jax.numpy as jnp
from jax import lax
from jax.experimental import pallas as pl
from jax.experimental.pallas import tpu as pltpu

F32 = jnp.float32
BF16 = jnp.bfloat16
LANES = 128
NT = (((1,), (1,)), ((), ()))


def _layernorm(x, eps=1e-5):
    m = jnp.mean(x, axis=-1, keepdims=True)
    d = x - m
    v = jnp.mean(d * d, axis=-1, keepdims=True)
    return d / jnp.sqrt(v + eps)


def _pick_rows(parts, row):
    bit = 1
    while len(parts) > 1:
        take_lo = (row & bit) == 0
        parts = [jnp.where(take_lo, parts[2 * i], parts[2 * i + 1]) for i in range(len(parts) // 2)]
        bit *= 2
    return parts[0]


def make_kernel(depth=8, kv_q0=16, w_q0=128, order="kvkv", nobc=True, compute=True, mode="batch"):
    NSEM = 16
    NS = 4
    assert depth < NSEM and depth <= 12

    def body(x_hbm, k_hbm, v_hbm, wq_hbm, wo_hbm, wr_hbm, wg_hbm, wu_hbm, wd_hbm, c_hbm, wm_hbm,
             out_ref,
             x_buf, c_buf, wr_buf, kbuf, vbuf, wm_buf, wq_buf, wo_buf, wg_buf, wu_buf, wd_buf,
             mod_scr, q_scr, s_scr, o_scr, a_scr, sems, small_sems):
        B, D = x_buf.shape
        _, H, S, Dh = k_hbm.shape
        W = min(4096, max(256, S // 4))
        T = W // LANES
        n_mod, n_q, n_f = wm_buf.shape[0], wq_buf.shape[0], wg_buf.shape[0]
        n_mod1 = 2 * D // LANES
        hb = B // 2
        scale = Dh ** -0.5

        def start_split(src, dst, n_rows, n_q0, sem):
            n1 = n_rows - n_q0
            pltpu.make_async_copy(src(0, n1), dst(0, n1), sem).start(priority=1)
            if n_q0:
                pltpu.make_async_copy(src(n1, n_q0), dst(n1, n_q0), sem).start(priority=0)

        def w_start(hbm, buf, i, sem):
            col = pl.ds(pl.multiple_of(i * LANES, LANES), LANES)
            start_split(lambda r, n: hbm.at[pl.ds(r, n), col],
                        lambda r, n: buf.at[i, pl.ds(r, n), :], D, w_q0, sem)

        def w_wait(buf, i, sem):
            pltpu.make_async_copy(buf.at[i], buf.at[i], sem).wait()

        def kv_start(hbm, buf, p, half, sem):
            h = p // T
            r0 = (S - W) + (p % T) * LANES
            bs = pl.ds(half * hb, hb)
            if mode == "batch":
                src = lambda r, n: hbm.at[bs, h, pl.ds(pl.multiple_of(r0 + r, 8), n), :]
            else:
                src = lambda r, n: hbm.at[h // 2, pl.ds((h % 2) * 8 + half * hb, hb), pl.ds(pl.multiple_of(r0 + r, 8), n), :]
            start_split(src, lambda r, n: buf.at[p % NS, bs, pl.ds(r, n), :], LANES, kv_q0, sem)

        def kv_wait(buf, p, half, sem):
            dst = buf.at[p % NS, pl.ds(half * hb, hb)]
            pltpu.make_async_copy(dst, dst, sem).wait()

        def weights(hbm, buf, first, steps):
            return (steps, 1,
                    lambda it, u, sem: w_start(hbm, buf, first + it, sem),
                    lambda it, u, sem: w_wait(buf, first + it, sem))

        def one_sided(hbm, buf, p0):
            return (2 * T, 4,
                    lambda it, u, sem: kv_start(hbm, buf, p0 + 2 * it + u // 2, u % 2, sem),
                    lambda it, u, sem: kv_wait(buf, p0 + 2 * it + u // 2, u % 2, sem))

        if order == "kvkv":
            kinds = [("k", 0), ("v", 0), ("k", 1), ("v", 1)]
        elif order == "vkvk":
            kinds = [("v", 0), ("k", 0), ("v", 1), ("k", 1)]
        elif order == "kkvv":
            kinds = [("k", 0), ("k", 1), ("v", 0), ("v", 1)]
        elif order == "vvkk":
            kinds = [("v", 0), ("v", 1), ("k", 0), ("k", 1)]

        def main_start(it, u, sem):
            kind, half = kinds[u]
            if kind == "k":
                kv_start(k_hbm, kbuf, it + T, half, sem)
            else:
                kv_start(v_hbm, vbuf, it, half, sem)

        def main_wait(it, u, sem):
            kind, half = kinds[u]
            if kind == "k":
                kv_wait(kbuf, it + T, half, sem)
            else:
                kv_wait(vbuf, it, half, sem)

        gate_up = (2 * n_f, 2,
                   lambda it, u, sem: w_start((wg_hbm, wu_hbm)[u], (wg_buf, wu_buf)[u], it, sem),
                   lambda it, u, sem: w_wait((wg_buf, wu_buf)[u], it, sem))
        phases = [
            weights(wm_hbm, wm_buf, 0, n_mod1),
            weights(wq_hbm, wq_buf, 0, n_q),
            one_sided(k_hbm, kbuf, 0),
            (4 * T * (H - 1), 4, main_start, main_wait),
            one_sided(v_hbm, vbuf, (H - 1) * T),
            weights(wo_hbm, wo_buf, 0, n_q),
            weights(wm_hbm, wm_buf, n_mod1, n_mod - n_mod1),
            gate_up,
            weights(wd_hbm, wd_buf, 0, n_f),
        ]
        bases = [0]
        for ph in phases:
            bases.append(bases[-1] + ph[0])

        def sem_of(t):
            return sems.at[t % NSEM]

        def advance(ph, it, u, unroll=None):
            steps, un, start, wait = phases[ph]
            unroll = unroll or un
            i = it * unroll + u
            t = bases[ph] + i
            wait(it * (unroll // un) + u // un, u % un, sem_of(t))
            nxt = sem_of(t + depth)
            ahead = u + depth

            @pl.when(i + depth < steps)
            def _():
                start(it * (unroll // un) + ahead // un, ahead % un, nxt)

            if ph + 1 < len(phases):
                _, un2, start2, _ = phases[ph + 1]
                assert unroll % un2 == 0 and steps % un2 == 0

                @pl.when(i + depth >= steps)
                def _():
                    start2(it * (unroll // un2) + ahead // un2 - steps // un2, ahead % un2, nxt)

        for t in range(depth):
            ph = max(p for p in range(len(phases)) if bases[p] <= t)
            un = phases[ph][1]
            phases[ph][2]((t - bases[ph]) // un, (t - bases[ph]) % un, sem_of(t))
            if t == 0:
                small = [pltpu.make_async_copy(s, d, small_sems.at[n])
                         for n, (s, d) in enumerate(((c_hbm, c_buf), (x_hbm, x_buf), (wr_hbm, wr_buf)))]
                for cp in small:
                    cp.start()
        small[0].wait()
        c = c_buf[...].astype(F32)
        sc = (c * jax.nn.sigmoid(c)).astype(BF16)

        def mod_step(ph, first):
            def step(i, carry):
                advance(ph, i, 0)
                col = pl.ds(pl.multiple_of((first + i) * LANES, LANES), LANES)
                mod_scr[:, col] = jnp.dot(sc, wm_buf[first + i], preferred_element_type=F32)
                return carry
            return step

        lax.fori_loop(0, n_mod1, mod_step(0, 0), 0)
        small[1].wait()
        x = x_buf[...].astype(F32)
        h = (_layernorm(x) * (1.0 + mod_scr[:, D:2 * D]) + mod_scr[:, 0:D]).astype(BF16)

        def q_step(it, carry):
            for u in range(4):
                advance(1, it, u, unroll=4)
                i = it * 4 + u
                q_scr[pl.ds(pl.multiple_of(i * B, B), B), :] = jnp.dot(h, wq_buf[i], preferred_element_type=F32)
            return carry

        lax.fori_loop(0, n_q // 4, q_step, 0)

        R = 2 * B
        row = lax.broadcasted_iota(jnp.int32, (R, LANES), 0)
        if mode == "batch":
            pair = row % B
        else:
            pair = row // 2
        low_half = pair < hb
        neg_inf = jnp.full((R, LANES), -jnp.inf, F32)
        zeros = jnp.zeros((R, LANES), F32)

        def load_q(g):
            if mode == "batch":
                return q_scr[pl.ds(pl.multiple_of(g * R, R), R), :].astype(BF16)
            return q_scr[pl.ds((g % 2) * R * B + g // 2, R, stride=B), :].astype(BF16)

        def qk(q, p, half):
            parts = [lax.dot_general(q, kbuf[p % NS, half * hb + n], NT, preferred_element_type=F32)
                     for n in range(hb)]
            return _pick_rows(parts, pair)

        def pv(prob, p, half):
            parts = [jnp.dot(prob, vbuf[p % NS, half * hb + n], preferred_element_type=F32)
                     for n in range(hb)]
            return _pick_rows(parts, pair)

        def probs(g, j, m):
            return jnp.exp((s_scr[g % 2, j] - m) * scale)

        def finish(g, l, acc):
            o = acc / jnp.sum(l, axis=-1, keepdims=True)
            if mode == "batch":
                o_scr[pl.ds(pl.multiple_of(g * R, R), R), :] = o
            else:
                o_scr[pl.ds((g % 2) * R * B + g // 2, R, stride=B), :] = o

        def row_max(m):
            return jnp.broadcast_to(jnp.max(m, axis=-1, keepdims=True), m.shape)

        q0 = load_q(0)

        def first_round(it, m):
            for jj in range(2):
                j = 2 * it + jj
                halves = []
                for half in range(2):
                    advance(2, it, 2 * jj + half)
                    halves.append(qk(q0, j, half))
                s = jnp.where(low_half, *halves)
                s_scr[0, j] = s
                m = jnp.maximum(m, s)
            return m

        m_prev = row_max(lax.fori_loop(0, T // 2, first_round, neg_inf))

        def main_round(g, m_prev):
            q = load_q(g + 1)

            def tile_row(j, carry):
                m, l, acc = carry
                it = g * T + j
                if not compute:
                    for u in range(4):
                        advance(3, it, u)
                    return carry
                prob = probs(g, j, m_prev)
                prob16 = prob.astype(BF16)
                ss, oo = [], []
                for u, (kind, half) in enumerate(kinds):
                    advance(3, it, u)
                    if kind == "k":
                        ss.append(qk(q, it + T, half))
                    else:
                        oo.append(pv(prob16, it, half))
                s = jnp.where(low_half, *ss)
                s_scr[(g + 1) % 2, j] = s
                return jnp.maximum(m, s), l + prob, acc + jnp.where(low_half, *oo)

            m, l, acc = lax.fori_loop(0, T, tile_row, (neg_inf, zeros, zeros))
            finish(g, l, acc)
            return row_max(m)

        m_prev = lax.fori_loop(0, H - 1, main_round, m_prev)

        def last_round(it, carry):
            l, acc = carry
            for jj in range(2):
                j = 2 * it + jj
                prob = probs(H - 1, j, m_prev)
                prob16 = prob.astype(BF16)
                halves = []
                for half in range(2):
                    advance(4, it, 2 * jj + half)
                    halves.append(pv(prob16, (H - 1) * T + j, half))
                l = l + prob
                acc = acc + jnp.where(low_half, *halves)
            return l, acc

        finish(H - 1, *lax.fori_loop(0, T // 2, last_round, (zeros, zeros)))

        def o_step(i, acc):
            advance(5, i, 0)
            o = o_scr[pl.ds(pl.multiple_of(i * B, B), B), :].astype(BF16)
            return acc + lax.dot_general(o, wo_buf[i], NT, preferred_element_type=F32)

        attn = lax.fori_loop(0, n_q, o_step, jnp.zeros((B, D), F32))

        def mod2_step(it, carry):
            for u in range(2):
                advance(6, it, u, unroll=2)
                i = n_mod1 + 2 * it + u
                col = pl.ds(pl.multiple_of(i * LANES, LANES), LANES)
                mod_scr[:, col] = jnp.dot(sc, wm_buf[i], preferred_element_type=F32)
            return carry

        lax.fori_loop(0, (n_mod - n_mod1) // 2, mod2_step, 0)
        x1 = x + mod_scr[:, 2 * D:3 * D] * attn
        h2 = _layernorm(x1) * (1.0 + mod_scr[:, 4 * D:5 * D]) + mod_scr[:, 3 * D:4 * D]
        h2b = h2.astype(BF16)

        def gu_step(f, carry):
            advance(7, f, 0)
            g = jnp.dot(h2b, wg_buf[f], preferred_element_type=F32)
            advance(7, f, 1)
            u = jnp.dot(h2b, wu_buf[f], preferred_element_type=F32)
            a_scr[f] = g * jax.nn.sigmoid(g) * u
            return carry

        lax.fori_loop(0, n_f, gu_step, 0)

        small[2].wait()
        wr = wr_buf[...].astype(F32).reshape(1, D)
        r_sel = jax.nn.sigmoid(jnp.sum(h2b.astype(F32) * wr, axis=-1, keepdims=True))
        gb = mod_scr[:, 5 * D:6 * D]

        def down_step(f, acc):
            advance(8, f, 0)
            return acc + lax.dot_general(a_scr[f].astype(BF16), wd_buf[f], NT, preferred_element_type=F32)

        y = lax.fori_loop(0, n_f, down_step, jnp.zeros((B, D), F32))
        out_ref[...] = (x1 + gb * (h2 + (h2 * 0.0 + y * r_sel))).astype(out_ref.dtype)

    def fn(A_x, A_k_cache, A_v_cache, A_wq, A_wo, B_x, B_w_r, B_w_gate, B_w_up, B_w_down, c, w_mod):
        del B_x
        B, Sq, D = A_x.shape
        _, H, S, Dh = A_k_cache.shape
        Hq = A_wq.shape[1] // Dh
        F = B_w_gate.shape[1]
        W = min(4096, max(256, S // 4))
        chunks = lambda n: pltpu.VMEM((n // LANES, D, LANES), BF16)
        out = pl.pallas_call(
            body,
            out_shape=jax.ShapeDtypeStruct((B, D), A_x.dtype),
            in_specs=[pl.BlockSpec(memory_space=pltpu.HBM)] * 11,
            out_specs=pl.BlockSpec(memory_space=pltpu.VMEM),
            scratch_shapes=[
                pltpu.VMEM((B, D), BF16), pltpu.VMEM((B, D), BF16), pltpu.VMEM((D,), BF16),
                pltpu.VMEM((NS, B, LANES, Dh), BF16), pltpu.VMEM((NS, B, LANES, Dh), BF16),
                chunks(w_mod.shape[1]), chunks(Hq * Dh), chunks(Hq * Dh), chunks(F), chunks(F), chunks(F),
                pltpu.VMEM((B, w_mod.shape[1]), F32),
                pltpu.VMEM((Hq * B, Dh), F32),
                pltpu.VMEM((2, W // LANES, 2 * B, LANES), F32),
                pltpu.VMEM((Hq * B, Dh), F32),
                pltpu.VMEM((F // LANES, B, LANES), F32),
                pltpu.SemaphoreType.DMA((NSEM,)),
                pltpu.SemaphoreType.DMA((3,)),
            ],
            compiler_params=pltpu.CompilerParams(
                vmem_limit_bytes=64 * 1024 * 1024, disable_bounds_checks=nobc),
        )(A_x.reshape(B, D), A_k_cache, A_v_cache, A_wq, A_wo.T, B_w_r, B_w_gate, B_w_up, B_w_down.T, c, w_mod)
        return out.reshape(B, Sq, D)

    return fn


_kernel = make_kernel()


@jax.jit
def pallas_adaLN_cond__sliding_block_cached__moe_arch_mod__decode_kernel(
    A_x: jax.Array,
    A_k_cache: jax.Array,
    A_v_cache: jax.Array,
    A_wq: jax.Array,
    A_wo: jax.Array,
    B_x: jax.Array,
    B_w_r: jax.Array,
    B_w_gate: jax.Array,
    B_w_up: jax.Array,
    B_w_down: jax.Array,
    c: jax.Array,
    w_mod: jax.Array,
):
    return _kernel(A_x, A_k_cache, A_v_cache, A_wq, A_wo, B_x, B_w_r, B_w_gate, B_w_up, B_w_down, c, w_mod)
```

```python
import contextlib

import jax
import jax.numpy as jnp
from jax import lax
from jax.experimental import pallas as pl
from jax.experimental.pallas import tpu as pltpu

F32 = jnp.float32
BF16 = jnp.bfloat16
LANES = 128
NT = (((1,), (1,)), ((), ()))


def _log2(n):
    assert n & (n - 1) == 0
    return n.bit_length() - 1


def _div(i, n):
    return i // n if isinstance(i, int) else lax.shift_right_logical(i, jnp.int32(_log2(n)))


def _mod(i, n):
    return i % n if isinstance(i, int) else i & (n - 1)


def _aligned(i, n):
    return i if isinstance(i, int) else pl.multiple_of(i, n)


def _layernorm(x, eps=1e-5):
    m = jnp.mean(x, axis=-1, keepdims=True)
    d = x - m
    v = jnp.mean(d * d, axis=-1, keepdims=True)
    return d / jnp.sqrt(v + eps)


def _pick(parts, owner, bit=1):
    while len(parts) > 1:
        lo = (owner & bit) == 0
        parts = [jnp.where(lo, parts[2 * i], parts[2 * i + 1]) for i in range(len(parts) // 2)]
        bit *= 2
    return parts[0]


def make_kernel(depth=8, seg=32, n0=4, w_q0=64, nobc=True, compute=True, scopes=False, wdepth=None):
    NSEM = 32
    NS = 8
    assert depth < NSEM
    scope = jax.named_scope if scopes else (lambda name: contextlib.nullcontext())

    def tile(buf, *idx):
        return pltpu.bitcast(buf.bitcast(jnp.uint32)[idx], BF16)

    def body(x_hbm, k_hbm, v_hbm, wq_hbm, wo_hbm, wr_hbm, wg_hbm, wu_hbm, wd_hbm, c_hbm, wm_hbm,
             out_ref,
             x_buf, c_buf, wr_buf, kv_buf, wm_buf, wq_buf, wo_buf, wg_buf, wu_buf, wd_buf,
             mod_scr, q_scr, s_scr, o_scr, a_scr, sems, small_sems):
        B, D = x_buf.shape
        _, H, S, Dh = k_hbm.shape
        W = min(4096, max(256, S // 4))
        T = W // LANES
        n_mod, n_q, n_f = wm_buf.shape[0], wq_buf.shape[0], wg_buf.shape[0]
        n_mod1 = 2 * D // LANES
        U = LANES // seg
        assert depth // U + 3 <= NS
        scale = Dh ** -0.5

        def w_start(hbm, buf, i, sem):
            col = pl.ds(_aligned(i * LANES, LANES), LANES)
            for r, n, prio in ((0, D - w_q0, 1), (D - w_q0, w_q0, 0)):
                if n:
                    pltpu.make_async_copy(hbm.at[pl.ds(r, n), col], buf.at[i, pl.ds(r, n), :], sem).start(priority=prio)

        def w_wait(sem):
            pltpu.make_async_copy(wq_buf.at[0], wq_buf.at[0], sem).wait()

        def kv_start(n, u, sem):
            b = _div(n, 2 * T)
            rows = pl.ds(_aligned((S - W) + _mod(n, T) * LANES + u * seg, 8), seg)

            def go(hbm):
                for h, nh, prio in ((0, H - n0, 1), (H - n0, n0, 0)):
                    if nh:
                        pltpu.make_async_copy(hbm.at[b, pl.ds(h, nh), rows, :],
                                              kv_buf.at[_mod(n, NS), pl.ds(h, nh), pl.ds(u * seg, seg), :],
                                              sem).start(priority=prio)

            is_v = _mod(_div(n, T), 2)
            if isinstance(is_v, int):
                go(v_hbm if is_v else k_hbm)
            else:
                pl.when(is_v == 0)(lambda: go(k_hbm))
                pl.when(is_v == 1)(lambda: go(v_hbm))

        def kv_wait(sem):
            dst = kv_buf.at[0, :, pl.ds(0, seg)]
            pltpu.make_async_copy(dst, dst, sem).wait()

        def weights(hbm, buf, first, steps):
            return (steps, 1, lambda i, u, sem: w_start(hbm, buf, first + i, sem), w_wait)

        phases = [
            weights(wm_hbm, wm_buf, 0, n_mod1),
            weights(wq_hbm, wq_buf, 0, n_q),
            (B * 2 * T * U, U, kv_start, kv_wait),
            weights(wo_hbm, wo_buf, 0, n_q),
            weights(wm_hbm, wm_buf, n_mod1, n_mod - n_mod1),
            (2 * n_f, 2, lambda i, u, sem: w_start((wg_hbm, wu_hbm)[u], (wg_buf, wu_buf)[u], i, sem), w_wait),
            weights(wd_hbm, wd_buf, 0, n_f),
        ]
        bases = [0]
        for ph in phases:
            bases.append(bases[-1] + ph[0])

        def in_phase(t0, stride, it, n_it, act):
            lo, hi = t0, t0 + stride * (n_it - 1)
            for p, (steps, group, _, _) in enumerate(phases):
                first, end = bases[p], bases[p + 1]
                if hi < first or lo >= end:
                    continue
                assert n_it == 1 or stride % group == 0
                i, u = (t0 - first) // group + (stride // group) * it, (t0 - first) % group
                t = t0 + stride * it
                conds = ([t >= first] if lo < first else []) + ([t < end] if hi >= end else [])
                if not conds:
                    act(p, i, u)
                else:
                    cond = conds[0] if len(conds) == 1 else jnp.logical_and(*conds)
                    pl.when(cond)(lambda p=p, i=i, u=u: act(p, i, u))

        def issue(t0, stride=1, it=0, n_it=1):
            sem = sems.at[_mod(t0 + stride * it, NSEM)]
            in_phase(t0, stride, it, n_it, lambda p, i, u: phases[p][2](i, u, sem))

        def advance(t0, stride=1, it=0, n_it=1):
            sem = sems.at[_mod(t0 + stride * it, NSEM)]
            in_phase(t0, stride, it, n_it, lambda p, i, u: phases[p][3](sem))
            issue(t0 + depth, stride, it, n_it)

        with scope("prologue"):
            for t in range(depth):
                issue(t)
                if t == 0:
                    small = [pltpu.make_async_copy(s, d, small_sems.at[n])
                             for n, (s, d) in enumerate(((c_hbm, c_buf), (x_hbm, x_buf), (wr_hbm, wr_buf)))]
                    for cp in small:
                        cp.start()
            small[0].wait()
            c = c_buf[...].astype(F32)
            sc = (c * jax.nn.sigmoid(c)).astype(BF16)

        def modulation(t0, first, n, unroll):
            def step(it, carry):
                for u in range(unroll):
                    advance(t0 + u, unroll, it, n // unroll)
                    i = first + it * unroll + u
                    col = pl.ds(pl.multiple_of(i * LANES, LANES), LANES)
                    mod_scr[:, col] = jnp.dot(sc, tile(wm_buf, i), preferred_element_type=F32)
                return carry
            lax.fori_loop(0, n // unroll, step, 0)

        with scope("A1"):
            modulation(bases[0], 0, n_mod1, 1)
        small[1].wait()
        x = x_buf[...].astype(F32)
        h = (_layernorm(x) * (1.0 + mod_scr[:, D:2 * D]) + mod_scr[:, 0:D]).astype(BF16)

        def q_step(it, carry):
            for u in range(U):
                advance(bases[1] + u, U, it, n_q // U)
                i = it * U + u
                q_scr[pl.ds(pl.multiple_of(i * B, B), B), :] = jnp.dot(h, tile(wq_buf, i), preferred_element_type=F32)
            return carry

        with scope("A2"):
            lax.fori_loop(0, n_q // U, q_step, 0)

        R = 16
        G = R // 2
        per_step = H // U
        owner = lax.broadcasted_iota(jnp.int32, (R, LANES), 0) // 2
        neg_inf = jnp.full((R, LANES), -jnp.inf, F32)
        zeros = jnp.zeros((R, LANES), F32)
        halves = range(H // G)

        def tile_row(n, product):
            parts = []
            for u in range(U):
                advance(bases[2] + U + u, U, n, B * 2 * T)
                if compute:
                    parts += [product(hd // G, tile(kv_buf, _mod(n, NS), hd))
                              for hd in range(u * per_step, (u + 1) * per_step)]
            if not compute:
                return [zeros for i in halves]
            return [_pick(parts[i * G:(i + 1) * G], owner) for i in halves]

        for u in range(U):
            advance(bases[2] + u)

        def batch(b, carry):
            q_rows = [pl.ds(i * R * B + b, R, stride=B) for i in halves]
            q = [q_scr[r, :].astype(BF16) for r in q_rows]

            def scores(j, m):
                s = tile_row(b * 2 * T + j,
                             lambda i, k: lax.dot_general(q[i], k, NT, preferred_element_type=F32))
                for i in halves:
                    s_scr[j, i] = s[i]
                return [jnp.maximum(m[i], s[i]) for i in halves]

            m = lax.fori_loop(0, T, scores, [neg_inf for i in halves])
            m = [jnp.broadcast_to(jnp.max(mi, axis=-1, keepdims=True), mi.shape) for mi in m]

            def values(j, carry):
                l, acc = carry
                p = [jnp.exp((s_scr[j, i] - m[i]) * scale) for i in halves]
                p16 = [pi.astype(BF16) for pi in p]
                o = tile_row(b * 2 * T + T + j,
                             lambda i, v: jnp.dot(p16[i], v, preferred_element_type=F32))
                return [l[i] + p[i] for i in halves], [acc[i] + o[i] for i in halves]

            l, acc = lax.fori_loop(0, T, values, ([zeros for i in halves], [zeros for i in halves]))
            for i in halves:
                o_scr[q_rows[i], :] = acc[i] / jnp.sum(l[i], axis=-1, keepdims=True)
            return carry

        with scope("B"):
            lax.fori_loop(0, B, batch, 0)

        def o_chunk(i):
            o = o_scr[pl.ds(_aligned(i * B, B), B), :].astype(BF16)
            return lax.dot_general(o, tile(wo_buf, i), NT, preferred_element_type=F32)

        def o_step(i, acc):
            advance(bases[3] + U, 1, i, n_q)
            return acc + o_chunk(i)

        with scope("C1"):
            attn = lax.fori_loop(0, n_q, o_step, jnp.zeros((B, D), F32))

        lag = U
        n_mod2 = n_mod - n_mod1

        def mod2_step(it, carry):
            for u in range(2):
                advance(bases[4] + lag + u, 2, it, n_mod2 // 2)
                i = n_mod1 + 2 * it + u
                col = pl.ds(pl.multiple_of(i * LANES, LANES), LANES)
                mod_scr[:, col] = jnp.dot(sc, tile(wm_buf, i), preferred_element_type=F32)
            return carry

        with scope("C2"):
            lax.fori_loop(0, n_mod2 // 2, mod2_step, 0)
        x1 = x + mod_scr[:, 2 * D:3 * D] * attn
        h2 = _layernorm(x1) * (1.0 + mod_scr[:, 4 * D:5 * D]) + mod_scr[:, 3 * D:4 * D]
        h2b = h2.astype(BF16)

        def gu_chunk(f):
            g = jnp.dot(h2b, tile(wg_buf, f), preferred_element_type=F32)
            u = jnp.dot(h2b, tile(wu_buf, f), preferred_element_type=F32)
            a_scr[f] = g * jax.nn.sigmoid(g) * u

        for f in range(lag // 2):
            gu_chunk(f)

        def gu_step(it, carry):
            n_it = n_f - lag // 2
            advance(bases[5] + lag, 2, it, n_it)
            advance(bases[5] + lag + 1, 2, it, n_it)
            gu_chunk(it + lag // 2)
            return carry

        with scope("C3"):
            lax.fori_loop(0, n_f - lag // 2, gu_step, 0)

        small[2].wait()
        wr = wr_buf[...].astype(F32).reshape(1, D)
        r_sel = jax.nn.sigmoid(jnp.sum(h2b.astype(F32) * wr, axis=-1, keepdims=True))
        gb = mod_scr[:, 5 * D:6 * D]

        def down_step(f, acc):
            advance(bases[6], 1, f, n_f)
            return acc + lax.dot_general(a_scr[f].astype(BF16), tile(wd_buf, f), NT, preferred_element_type=F32)

        with scope("C4"):
            y = lax.fori_loop(0, n_f, down_step, jnp.zeros((B, D), F32))
        out_ref[...] = (x1 + gb * (h2 + (h2 * 0.0 + y * r_sel))).astype(out_ref.dtype)

    def fn(A_x, A_k_cache, A_v_cache, A_wq, A_wo, B_x, B_w_r, B_w_gate, B_w_up, B_w_down, c, w_mod):
        del B_x
        B, Sq, D = A_x.shape
        _, H, S, Dh = A_k_cache.shape
        Hq = A_wq.shape[1] // Dh
        F = B_w_gate.shape[1]
        W = min(4096, max(256, S // 4))
        chunks = lambda n: pltpu.VMEM((n // LANES, D, LANES), BF16)
        out = pl.pallas_call(
            body,
            out_shape=jax.ShapeDtypeStruct((B, D), A_x.dtype),
            in_specs=[pl.BlockSpec(memory_space=pltpu.HBM)] * 11,
            out_specs=pl.BlockSpec(memory_space=pltpu.VMEM),
            scratch_shapes=[
                pltpu.VMEM((B, D), BF16), pltpu.VMEM((B, D), BF16), pltpu.VMEM((D,), BF16),
                pltpu.VMEM((NS, H, LANES, Dh), BF16),
                chunks(w_mod.shape[1]), chunks(Hq * Dh), chunks(Hq * Dh), chunks(F), chunks(F), chunks(F),
                pltpu.VMEM((B, w_mod.shape[1]), F32),
                pltpu.VMEM((Hq * B, Dh), F32),
                pltpu.VMEM((W // LANES, Hq // 16, 16, LANES), F32),
                pltpu.VMEM((Hq * B, Dh), F32),
                pltpu.VMEM((F // LANES, B, LANES), F32),
                pltpu.SemaphoreType.DMA((NSEM,)),
                pltpu.SemaphoreType.DMA((3,)),
            ],
            compiler_params=pltpu.CompilerParams(
                vmem_limit_bytes=64 * 1024 * 1024, disable_bounds_checks=nobc),
        )(A_x.reshape(B, D), A_k_cache, A_v_cache, A_wq, A_wo.T, B_w_r, B_w_gate, B_w_up, B_w_down.T, c, w_mod)
        return out.reshape(B, Sq, D)

    return fn


_kernel = make_kernel()


@jax.jit
def pallas_adaLN_cond__sliding_block_cached__moe_arch_mod__decode_kernel(
    A_x: jax.Array,
    A_k_cache: jax.Array,
    A_v_cache: jax.Array,
    A_wq: jax.Array,
    A_wo: jax.Array,
    B_x: jax.Array,
    B_w_r: jax.Array,
    B_w_gate: jax.Array,
    B_w_up: jax.Array,
    B_w_down: jax.Array,
    c: jax.Array,
    w_mod: jax.Array,
):
    return _kernel(A_x, A_k_cache, A_v_cache, A_wq, A_wo, B_x, B_w_r, B_w_gate, B_w_up, B_w_down, c, w_mod)
```

```python
import contextlib
import math

import jax
import jax.numpy as jnp
from jax import lax
from jax.experimental import pallas as pl
from jax.experimental.pallas import tpu as pltpu

F32 = jnp.float32
BF16 = jnp.bfloat16
LANES = 128
NT = (((1,), (1,)), ((), ()))


def _log2(n):
    assert n & (n - 1) == 0
    return n.bit_length() - 1


def _div(i, n):
    return i // n if isinstance(i, int) else lax.shift_right_logical(i, jnp.int32(_log2(n)))


def _mod(i, n):
    return i % n if isinstance(i, int) else i & (n - 1)


def _small_div(i, n, limit):
    if isinstance(i, int):
        return i // n
    magic = (1 << 16) // n + 1
    assert all((k * magic) >> 16 == k // n for k in range(limit))
    return lax.shift_right_logical(i * magic, jnp.int32(16))


def _aligned(i, n):
    return i if isinstance(i, int) else pl.multiple_of(i, n)


def _layernorm(x, eps=1e-5):
    m = jnp.mean(x, axis=-1, keepdims=True)
    d = x - m
    v = jnp.mean(d * d, axis=-1, keepdims=True)
    return d / jnp.sqrt(v + eps)


def _pick(parts, owner, bit=1):
    while len(parts) > 1:
        lo = (owner & bit) == 0
        parts = [jnp.where(lo, parts[2 * i], parts[2 * i + 1]) for i in range(len(parts) // 2)]
        bit *= 2
    return parts[0]


def make_kernel(depth=16, seg=16, n0=2, w_n0=1, wcols=512, mcols=384, d_q0=32, nobc=True, compute=True, scopes=False, pace=0, every=2, nosc=True):
    NSEM = 32
    NS = 8
    assert depth < NSEM
    scope = jax.named_scope if scopes else (lambda name: contextlib.nullcontext())

    def tile(buf, *idx):
        return pltpu.bitcast(buf.bitcast(jnp.uint32)[idx], BF16)

    def body(x_hbm, k_hbm, v_hbm, wq_hbm, wo_hbm, wr_hbm, wg_hbm, wu_hbm, wd_hbm, c_hbm, wm_hbm,
             out_ref,
             x_buf, c_buf, wr_buf, kv_buf, wm_buf, wq_buf, wo_buf, wg_buf, wu_buf, wd_buf,
             mod_scr, q_scr, s_scr, o_scr, a_scr, tail_scr, sems, small_sems):
        B, D = x_buf.shape
        _, H, S, Dh = k_hbm.shape
        W = min(4096, max(256, S // 4))
        T = W // LANES
        n_mod, n_q, n_f = wm_buf.shape[2] // LANES, wq_buf.shape[2] // LANES, wg_buf.shape[2] // LANES
        n_mod1 = 2 * D // LANES
        NSEG, SEG_ROWS = wq_buf.shape[:2]
        U = LANES // seg
        assert depth // U + 3 <= NS
        scale = Dh ** -0.5

        def w_start(hbm, buf, r, c0, cols, sem):
            rows = pl.ds(_aligned(r * 8, 8), 8)
            for s0, n, prio in ((0, NSEG - w_n0, 1), (NSEG - w_n0, w_n0, 0)):
                if n:
                    at = (pl.ds(s0, n), rows, pl.ds(_aligned(c0, LANES), cols))
                    pltpu.make_async_copy(hbm.at[at], buf.at[at], sem).start(priority=prio)

        def w_wait(buf, cols, sem):
            dst = buf.at[:, pl.ds(0, 8), pl.ds(0, cols)]
            pltpu.make_async_copy(dst, dst, sem).wait()

        def weights(arrays, c0, width, cols):
            n_cols = width // cols
            steps = SEG_ROWS // 8 * n_cols

            def start(i, u, sem):
                r = _small_div(i, n_cols, steps)
                w_start(*arrays[u], r, c0 + (i - r * n_cols) * cols, cols, sem)

            return steps * len(arrays), len(arrays), start, lambda sem: w_wait(arrays[0][1], cols, sem)

        def d_start(f, u, sem):
            col = pl.ds(_aligned(f * LANES, LANES), LANES)
            for r, n, prio in ((0, D // 2 - d_q0, 1), (D // 2 - d_q0, d_q0, 0)):
                if n:
                    rows = pl.ds(u * (D // 2) + r, n)
                    pltpu.make_async_copy(wd_hbm.at[rows, col], wd_buf.at[f, rows, :], sem).start(priority=prio)

        def d_wait(sem):
            dst = wd_buf.at[0, pl.ds(0, D // 2)]
            pltpu.make_async_copy(dst, dst, sem).wait()

        def col(buf, i, n=1):
            return buf[:, :, pl.ds(_aligned(i * n * LANES, LANES), n * LANES)].reshape(D, n * LANES)

        def kv_start(n, u, sem):
            b = _div(n, 2 * T)
            rows = pl.ds(_aligned((S - W) + _mod(n, T) * LANES + u * seg, 8), seg)

            def go(hbm):
                for h, nh, prio in ((0, H - n0, 1), (H - n0, n0, 0)):
                    if nh:
                        pltpu.make_async_copy(hbm.at[b, pl.ds(h, nh), rows, :],
                                              kv_buf.at[_mod(n, NS), pl.ds(h, nh), pl.ds(u * seg, seg), :],
                                              sem).start(priority=prio)

            is_v = _mod(_div(n, T), 2)
            if isinstance(is_v, int):
                go(v_hbm if is_v else k_hbm)
            else:
                pl.when(is_v == 0)(lambda: go(k_hbm))
                pl.when(is_v == 1)(lambda: go(v_hbm))

        def kv_wait(sem):
            dst = kv_buf.at[0, :, pl.ds(0, seg)]
            pltpu.make_async_copy(dst, dst, sem).wait()

        wq, wo, wg, wu, wm = (wq_hbm, wq_buf), (wo_hbm, wo_buf), (wg_hbm, wg_buf), (wu_hbm, wu_buf), (wm_hbm, wm_buf)
        phases = [weights([wm], 0, n_mod1 * LANES, mcols)]
        phases += [
            weights([wq], 0, n_q * LANES, wcols),
            weights([wm], n_mod1 * LANES, (n_mod - n_mod1) * LANES, mcols),
            weights([wo], 0, n_q * LANES, wcols),
            (B * 2 * T * U, U, kv_start, kv_wait),
            weights([wg], 0, n_f * LANES, wcols),
            weights([wu], 0, n_f * LANES, wcols),
            (2 * n_f, 2, d_start, d_wait),
        ]
        bases = [0]
        for ph in phases:
            bases.append(bases[-1] + ph[0])
        t_wq, t_wm2, t_wo, t_kv, t_wg, t_wu, t_wd = bases[1:-1]

        def in_phase(t0, stride, it, n_it, act, indexed=True):
            lo, hi = t0, t0 + stride * (n_it - 1)
            for p, (steps, group, _, _) in enumerate(phases):
                first, end = bases[p], bases[p + 1]
                if hi < first or lo >= end:
                    continue
                assert n_it == 1 or stride % group == 0 or not indexed
                i, u = (t0 - first) // group + (stride // group) * it, (t0 - first) % group
                t = t0 + stride * it
                conds = ([t >= first] if lo < first else []) + ([t < end] if hi >= end else [])
                if not conds:
                    act(p, i, u)
                else:
                    cond = conds[0] if len(conds) == 1 else jnp.logical_and(*conds)
                    pl.when(cond)(lambda p=p, i=i, u=u: act(p, i, u))

        def issue(t0, stride=1, it=0, n_it=1):
            sem = sems.at[_mod(t0 + stride * it, NSEM)]
            in_phase(t0, stride, it, n_it, lambda p, i, u: phases[p][2](i, u, sem))

        def advance(t0, stride=1, it=0, n_it=1):
            sem = sems.at[_mod(t0 + stride * it, NSEM)]
            in_phase(t0, stride, it, n_it, lambda p, i, u: phases[p][3](sem), indexed=False)
            issue(t0 + depth, stride, it, n_it)

        with scope("prologue"):
            for t in range(depth):
                issue(t)
                if t == 0:
                    small = [pltpu.make_async_copy(s, d, small_sems.at[n])
                             for n, (s, d) in enumerate(((c_hbm, c_buf), (x_hbm, x_buf), (wr_hbm, wr_buf)))]
                    for cp in small:
                        cp.start()
                if pace and t >= pace[0]:
                    pl.delay(pace[1])
            small[0].wait()
            c = c_buf[...].astype(F32)
            sc = (c * jax.nn.sigmoid(c)).astype(BF16)

        def stream(t0, t1, work=(), carry=None):
            cuts = {t0, t1}
            for first, n, every, fn in work:
                cuts |= {first, first + n * every}
            for b_ in bases:
                cuts |= {b_, b_ - depth}
            cuts = sorted(t for t in cuts if t0 <= t <= t1)
            for lo, hi in zip(cuts[:-1], cuts[1:]):
                job = [w for w in work if w[0] <= lo < w[0] + w[1] * w[2]]
                unroll = job[0][2] if job else 1
                for p, ph in enumerate(phases):
                    if bases[p] <= lo + depth < bases[p + 1]:
                        unroll = unroll * ph[1] // math.gcd(unroll, ph[1])

                def run(t, stride, it, n_it, carry):
                    advance(t, stride, it, n_it)
                    for first, n, every, fn in job:
                        if (t - first) % every == every - 1:
                            carry = fn((t - first) // every + (stride // every) * it, carry)
                    return carry

                n_it = (hi - lo) // unroll
                if n_it > 1:
                    def body_(it, carry):
                        for u in range(unroll):
                            carry = run(lo + u, unroll, it, n_it, carry)
                        return carry
                    carry = lax.fori_loop(0, n_it, body_, carry)
                else:
                    n_it = 0
                for t in range(lo + n_it * unroll, hi):
                    carry = run(t, unroll, 0, 1, carry)
            return carry

        def mod_chunk(first):
            def fn(i, carry):
                i = first + i
                mod_scr[:, pl.ds(_aligned(i * LANES, LANES), LANES)] = jnp.dot(sc, col(wm_buf, i), preferred_element_type=F32)
                return carry
            return fn

        with scope("A1"):
            stream(0, t_wq + 2 * n_mod1, [(t_wq, n_mod1, 2, mod_chunk(0))], 0)
        small[1].wait()
        x = x_buf[...].astype(F32)
        h = (_layernorm(x) * (1.0 + mod_scr[:, D:2 * D]) + mod_scr[:, 0:D]).astype(BF16)

        def q_chunk(i, carry):
            q = jnp.dot(h, col(wq_buf, i, 2), preferred_element_type=F32)
            for n in range(2):
                q_scr[pl.ds(_aligned((2 * i + n) * B, B), B), :] = q[:, n * LANES:(n + 1) * LANES]
            return carry

        with scope("A2"):
            n_mod2 = n_mod - n_mod1
            stream(t_wq + 2 * n_mod1, t_kv + U,
                   [(t_wm2, n_q // 2, (t_wo - t_wm2) // (n_q // 2), q_chunk), (t_wo, n_mod2, 2, mod_chunk(n_mod1))], 0)

        R = 16
        G = R // 2
        per_step = H // U
        owner = lax.broadcasted_iota(jnp.int32, (R, LANES), 0) // 2
        neg_inf = jnp.full((R, LANES), -jnp.inf, F32)
        zeros = jnp.zeros((R, LANES), F32)
        halves = range(H // G)

        def tile_row(n, product):
            parts = []
            for u in range(U):
                advance(t_kv + U + u, U, n, B * 2 * T)
                if compute and u % every == 0:
                    parts += [product(hd // G, tile(kv_buf, _mod(n, NS), hd))
                              for hd in range(u * per_step, (u + every) * per_step)]
            if not compute:
                return [zeros for i in halves]
            return [_pick(parts[i * G:(i + 1) * G], owner) for i in halves]

        def batch(b, carry):
            q_rows = [pl.ds(i * R * B + b, R, stride=B) for i in halves]
            q = [q_scr[r, :].astype(BF16) for r in q_rows]

            def scores(j, m):
                s = tile_row(b * 2 * T + j,
                             lambda i, k: lax.dot_general(q[i], k, NT, preferred_element_type=F32))
                for i in halves:
                    s_scr[j, i] = s[i]
                return [jnp.maximum(m[i], s[i]) for i in halves]

            m = lax.fori_loop(0, T, scores, [neg_inf for i in halves])
            m = [jnp.broadcast_to(jnp.max(mi, axis=-1, keepdims=True), mi.shape) for mi in m]

            def values(j, carry):
                l, acc = carry
                p = [jnp.exp((s_scr[j, i] - m[i]) * scale) for i in halves]
                p16 = [pi.astype(BF16) for pi in p]
                o = tile_row(b * 2 * T + T + j,
                             lambda i, v: jnp.dot(p16[i], v, preferred_element_type=F32))
                return [l[i] + p[i] for i in halves], [acc[i] + o[i] for i in halves]

            l, acc = lax.fori_loop(0, T, values, ([zeros for i in halves], [zeros for i in halves]))
            for i in halves:
                o_scr[q_rows[i], :] = acc[i] / jnp.sum(l[i], axis=-1, keepdims=True)
            return carry

        with scope("B"):
            lax.fori_loop(0, B, batch, 0)

        def o_chunk(i, acc):
            o = o_scr[pl.ds(_aligned(i * B, B), B), :].astype(BF16)
            return acc + lax.dot_general(o, col(wo_buf, i), NT, preferred_element_type=F32)

        with scope("C1"):
            t = t_wg + U
            attn = stream(t, t + 2 * n_q, [(t, n_q, 2, o_chunk)], jnp.zeros((B, D), F32))
        x1 = x + mod_scr[:, 2 * D:3 * D] * attn
        h2 = _layernorm(x1) * (1.0 + mod_scr[:, 4 * D:5 * D]) + mod_scr[:, 3 * D:4 * D]
        h2b = h2.astype(BF16)

        def gate_chunk(f, carry):
            g = jnp.dot(h2b, col(wg_buf, f), preferred_element_type=F32)
            a_scr[f] = g * jax.nn.sigmoid(g)
            return carry

        with scope("C2"):
            t = t + 2 * n_q
            assert t >= t_wu and t + 2 * n_f <= t_wd
            stream(t, t_wd, [(t, n_f, 2, gate_chunk)], 0)

        small[2].wait()
        wr = wr_buf[...].astype(F32).reshape(1, D)
        r_sel = jax.nn.sigmoid(jnp.sum(h2b.astype(F32) * wr, axis=-1, keepdims=True))
        gb = mod_scr[:, 5 * D:6 * D]
        tail_scr[0] = x1 + gb * (h2 + h2 * 0.0)
        tail_scr[1] = gb * r_sel

        def up(f):
            return (a_scr[f] * jnp.dot(h2b, col(wu_buf, f), preferred_element_type=F32)).astype(BF16)

        def down_step(f, carry):
            acc, a = carry
            advance(t_wd, 2, f, n_f)
            advance(t_wd + 1, 2, f, n_f)
            acc = acc + lax.dot_general(a, tile(wd_buf, f), NT, preferred_element_type=F32)
            return acc, up(jnp.minimum(f + 1, n_f - 1))

        with scope("C3"):
            y, a = lax.fori_loop(0, n_f - 1, down_step, (jnp.zeros((B, D), F32), up(0)))
            advance(t_wd + 2 * n_f - 2)
            advance(t_wd + 2 * n_f - 1)
            y = y + lax.dot_general(a, tile(wd_buf, n_f - 1), NT, preferred_element_type=F32)
        out_ref[...] = (tail_scr[0] + tail_scr[1] * y).astype(out_ref.dtype)

    def fn(A_x, A_k_cache, A_v_cache, A_wq, A_wo, B_x, B_w_r, B_w_gate, B_w_up, B_w_down, c, w_mod):
        del B_x
        B, Sq, D = A_x.shape
        _, H, S, Dh = A_k_cache.shape
        Hq = A_wq.shape[1] // Dh
        F = B_w_gate.shape[1]
        W = min(4096, max(256, S // 4))
        banded = lambda w: w.reshape(9, D // 9, w.shape[1])
        held = lambda n: pltpu.VMEM((9, D // 9, n), BF16)
        out = pl.pallas_call(
            body,
            out_shape=jax.ShapeDtypeStruct((B, D), A_x.dtype),
            in_specs=[pl.BlockSpec(memory_space=pltpu.HBM)] * 11,
            out_specs=pl.BlockSpec(memory_space=pltpu.VMEM),
            scratch_shapes=[
                pltpu.VMEM((B, D), BF16), pltpu.VMEM((B, D), BF16), pltpu.VMEM((D,), BF16),
                pltpu.VMEM((NS, H, LANES, Dh), BF16),
                held(w_mod.shape[1]), held(Hq * Dh), held(Hq * Dh), held(F), held(F),
                pltpu.VMEM((F // LANES, D, LANES), BF16),
                pltpu.VMEM((B, w_mod.shape[1]), F32),
                pltpu.VMEM((Hq * B, Dh), F32),
                pltpu.VMEM((W // LANES, Hq // 16, 16, LANES), F32),
                pltpu.VMEM((Hq * B, Dh), F32),
                pltpu.VMEM((F // LANES, B, LANES), F32),
                pltpu.VMEM((2, B, D), F32),
                pltpu.SemaphoreType.DMA((NSEM,)),
                pltpu.SemaphoreType.DMA((3,)),
            ],
            compiler_params=pltpu.CompilerParams(
                vmem_limit_bytes=64 * 1024 * 1024, disable_bounds_checks=nobc, disable_semaphore_checks=nosc),
        )(A_x.reshape(B, D), A_k_cache, A_v_cache, banded(A_wq), banded(A_wo.T), B_w_r,
          banded(B_w_gate), banded(B_w_up), B_w_down.T, c, banded(w_mod))
        return out.reshape(B, Sq, D)

    return fn


_kernel = make_kernel()


@jax.jit
def pallas_adaLN_cond__sliding_block_cached__moe_arch_mod__decode_kernel(
    A_x: jax.Array,
    A_k_cache: jax.Array,
    A_v_cache: jax.Array,
    A_wq: jax.Array,
    A_wo: jax.Array,
    B_x: jax.Array,
    B_w_r: jax.Array,
    B_w_gate: jax.Array,
    B_w_up: jax.Array,
    B_w_down: jax.Array,
    c: jax.Array,
    w_mod: jax.Array,
):
    return _kernel(A_x, A_k_cache, A_v_cache, A_wq, A_wo, B_x, B_w_r, B_w_gate, B_w_up, B_w_down, c, w_mod)
```

```python
import math

import jax
import jax.numpy as jnp
from jax import lax
from jax.experimental import pallas as pl
from jax.experimental.pallas import tpu as pltpu

F32 = jnp.float32
BF16 = jnp.bfloat16
LANES = 128
NT = (((1,), (1,)), ((), ()))

DEPTH = 16
KEYS = 16
KV_SLOTS = 4
BANDS = 9
Q_ROWS = 16


def _div(i, n, limit):
    if isinstance(i, int):
        return i // n
    if n & (n - 1) == 0:
        return lax.shift_right_logical(i, jnp.int32(n.bit_length() - 1))
    magic = (1 << 16) // n + 1
    assert all((k * magic) >> 16 == k // n for k in range(limit))
    return lax.shift_right_logical(i * magic, jnp.int32(16))


def _mod(i, n):
    assert n & (n - 1) == 0
    return i % n if isinstance(i, int) else i & (n - 1)


def _block(i, n, base=0, align=None):
    start = base + i * n
    return pl.ds(start if isinstance(start, int) else pl.multiple_of(start, align or n), n)


def _runs(total, urgent):
    runs, lo = [], 0
    for first, count in urgent:
        runs += [(lo, first - lo, 1), (first, count, 0)]
        lo = first + count
    return [run for run in runs + [(lo, total - lo, 1)] if run[1]]


def _layernorm(x, eps=1e-5):
    d = x - jnp.mean(x, axis=-1, keepdims=True)
    return d / jnp.sqrt(jnp.mean(d * d, axis=-1, keepdims=True) + eps)


def _silu(x):
    return x * jax.nn.sigmoid(x)


def _pick(parts, owner):
    bit = 1
    while len(parts) > 1:
        even = (owner & bit) == 0
        parts = [jnp.where(even, a, b) for a, b in zip(parts[0::2], parts[1::2])]
        bit *= 2
    return parts[0]


class _Stream:
    def __init__(self, phases, sems):
        self.phases, self.sems = phases, sems
        self.bases = [0]
        for phase in phases:
            self.bases.append(self.bases[-1] + phase[0])

    def _each(self, t0, stride, it, n_it, act):
        sem = self.sems.at[_mod(t0 + stride * it, DEPTH)]
        for phase, first, end in zip(self.phases, self.bases, self.bases[1:]):
            last = t0 + stride * (n_it - 1)
            if last < first or t0 >= end:
                continue
            group = phase[1]
            assert n_it == 1 or stride % group == 0
            assert t0 >= first or last < end
            run = lambda: act(phase, (t0 - first) // group + stride // group * it, (t0 - first) % group, sem)
            if t0 < first:
                pl.when(t0 + stride * it >= first)(run)
            elif last >= end:
                pl.when(t0 + stride * it < end)(run)
            else:
                run()

    def start(self, t0, stride=1, it=0, n_it=1):
        self._each(t0, stride, it, n_it, lambda phase, i, u, sem: phase[2](i, u, sem))

    def advance(self, t0, stride=1, it=0, n_it=1):
        def wait(phase, i, u, sem):
            target = phase[3](i, u)
            pltpu.make_async_copy(target, target, sem).wait()

        self._each(t0, stride, it, n_it, wait)
        self.start(t0 + DEPTH, stride, it, n_it)

    def run(self, t0, t1, work=(), carry=0):
        cuts = {t0, t1, *self.bases, *(base - DEPTH for base in self.bases)}
        for first, n, every, _ in work:
            assert t0 <= first and first + n * every <= t1
            cuts |= {first, first + n * every}
        cuts = sorted(t for t in cuts if t0 <= t <= t1)
        for lo, hi in zip(cuts, cuts[1:]):
            jobs = [job for job in work if job[0] <= lo < job[0] + job[1] * job[2]]
            unroll = math.lcm(*(job[2] for job in jobs), *(
                phase[1] for phase, first, end in zip(self.phases, self.bases, self.bases[1:])
                if first <= lo < end or first <= lo + DEPTH < end))

            def step(t, it, n_it, carry):
                self.advance(t, unroll, it, n_it)
                for first, _, every, fn in jobs:
                    if (t - first) % every == every - 1:
                        carry = fn((t - first) // every + unroll // every * it, carry)
                return carry

            n_it = (hi - lo) // unroll
            if n_it > 1:
                def body(it, carry):
                    for u in range(unroll):
                        carry = step(lo + u, it, n_it, carry)
                    return carry

                carry = lax.fori_loop(0, n_it, body, carry)
                lo += n_it * unroll
            for t in range(lo, hi):
                carry = step(t, 0, 1, carry)
        return carry


def _kernel(x_hbm, k_hbm, v_hbm, wq_hbm, wo_hbm, wr_hbm, wg_hbm, wu_hbm, wd_hbm, c_hbm, wm_hbm,
            out_ref,
            x_buf, c_buf, wr_buf, kv_buf, wm_buf, wq_buf, wo_buf, wg_buf, wu_buf, wd_buf,
            mod_scr, q_scr, s_scr, o_scr, g_scr, tail_scr, sems, small_sems):
    B, D = x_buf.shape
    _, H, S, Dh = k_hbm.shape
    W = min(4096, max(256, S // 4))
    T = W // LANES
    U = LANES // KEYS
    n_rows = B * 2 * T
    n_mod, n_q, n_f = (buf.shape[2] // LANES for buf in (wm_buf, wq_buf, wg_buf))
    n_mod1 = pl.cdiv(2 * D, LANES)
    assert DEPTH // U + 2 <= KV_SLOTS

    def banded(hbm, buf, chunk0, chunks, cols):
        n_cols = chunks * LANES // cols
        assert n_cols * cols == chunks * LANES
        steps = buf.shape[1] // 8 * n_cols

        def where(i):
            r = _div(i, n_cols, steps)
            return _block(r, 8), _block(i - r * n_cols, cols, chunk0 * LANES, LANES)

        def start(i, u, sem):
            for band, count, priority in _runs(BANDS, [(BANDS - 1, 1)]):
                at = (pl.ds(band, count), *where(i))
                pltpu.make_async_copy(hbm.at[at], buf.at[at], sem).start(priority=priority)

        return steps, 1, start, lambda i, u: buf.at[(slice(None), *where(i))]

    def kv_start(n, u, sem):
        keys = _block(_mod(n, T) * U + u, KEYS, S - W)

        def start_from(hbm):
            for head, count, priority in _runs(H, [(H // 2 - 1, 1), (H - 1, 1)]):
                pltpu.make_async_copy(
                    hbm.at[_div(n, 2 * T, n_rows), pl.ds(head, count), keys],
                    kv_buf.at[_mod(n, KV_SLOTS), pl.ds(head, count), _block(u, KEYS)],
                    sem).start(priority=priority)

        is_value = _mod(_div(n, T, n_rows), 2)
        if isinstance(is_value, int):
            start_from(v_hbm if is_value else k_hbm)
        else:
            pl.when(is_value == 0)(lambda: start_from(k_hbm))
            pl.when(is_value == 1)(lambda: start_from(v_hbm))

    def down_start(f, u, sem):
        for row, count, priority in _runs(D // 2, [(D // 2 - 16, 16)]):
            rows = pl.ds(u * (D // 2) + row, count)
            pltpu.make_async_copy(
                wd_hbm.at[rows, _block(f, LANES)], wd_buf.at[f, rows], sem).start(priority=priority)

    stream = _Stream([
        banded(wm_hbm, wm_buf, 0, n_mod1, 384),
        banded(wq_hbm, wq_buf, 0, n_q, 512),
        banded(wm_hbm, wm_buf, n_mod1, n_mod - n_mod1, 384),
        banded(wo_hbm, wo_buf, 0, n_q, 512),
        (n_rows * U, U, kv_start, lambda n, u: kv_buf.at[_mod(n, KV_SLOTS), :, _block(u, KEYS)]),
        banded(wg_hbm, wg_buf, 0, n_f, 512),
        banded(wu_hbm, wu_buf, 0, n_f, 512),
        (2 * n_f, 2, down_start, lambda f, u: wd_buf.at[f, _block(u, D // 2)]),
    ], sems)
    t_wq, t_wm2, t_wo, t_kv, t_wg, t_wu, t_wd = stream.bases[1:-1]

    def columns(buf, i, n=1):
        return buf[:, :, _block(i, n * LANES)].reshape(D, n * LANES)

    small = [pltpu.make_async_copy(src, dst, small_sems.at[n])
             for n, (src, dst) in enumerate(((c_hbm, c_buf), (x_hbm, x_buf), (wr_hbm, wr_buf)))]
    stream.start(0)
    for copy in small:
        copy.start()
    for t in range(1, DEPTH):
        stream.start(t)

    small[0].wait()
    cond = _silu(c_buf[...].astype(F32)).astype(BF16)

    def mod_chunk(first):
        def fn(i, carry):
            mod_scr[:, _block(first + i, LANES)] = jnp.dot(
                cond, columns(wm_buf, first + i), preferred_element_type=F32)
            return carry
        return fn

    def mod(i):
        return mod_scr[:, i * D:(i + 1) * D]

    t = t_wq + 2 * n_mod1
    stream.run(0, t, [(t_wq, n_mod1, 2, mod_chunk(0))])
    small[1].wait()
    x = x_buf[...].astype(F32)
    h = (_layernorm(x) * (1.0 + mod(1)) + mod(0)).astype(BF16)

    def q_chunk(i, carry):
        q = jnp.dot(h, columns(wq_buf, i, 2), preferred_element_type=F32)
        for n in range(2):
            q_scr[_block(2 * i + n, B), :] = q[:, n * LANES:(n + 1) * LANES]
        return carry

    stream.run(t, t_kv + U, [(t_wm2, n_q // 2, 3, q_chunk), (t_wo, n_mod - n_mod1, 2, mod_chunk(n_mod1))])

    G = Q_ROWS // 2
    groups = range(H // G)
    owner = lax.broadcasted_iota(jnp.int32, (Q_ROWS, LANES), 0) // 2
    scale = Dh ** -0.5

    def tile_row(n, product):
        parts = []
        for u in range(U):
            stream.advance(t_kv + U + u, U, n, n_rows)
            if u % 2 == 0:
                parts += [product(head // G, kv_buf[_mod(n, KV_SLOTS), head])
                          for head in range(u * H // U, (u + 2) * H // U)]
        return [_pick(parts[g * G:(g + 1) * G], owner) for g in groups]

    def attend(b, carry):
        rows = [pl.ds(g * Q_ROWS * B + b, Q_ROWS, stride=B) for g in groups]
        q = [q_scr[r, :].astype(BF16) for r in rows]

        def scores(j, m):
            s = tile_row(b * 2 * T + j,
                         lambda g, k: lax.dot_general(q[g], k, NT, preferred_element_type=F32))
            for g in groups:
                s_scr[j, g] = s[g]
            return [jnp.maximum(m[g], s[g]) for g in groups]

        m = lax.fori_loop(0, T, scores, [jnp.full((Q_ROWS, LANES), -jnp.inf, F32) for _ in groups])
        m = [jnp.broadcast_to(jnp.max(mg, axis=-1, keepdims=True), mg.shape) for mg in m]

        def values(j, carry):
            l, acc = carry
            p = [jnp.exp((s_scr[j, g] - m[g]) * scale) for g in groups]
            p16 = [pg.astype(BF16) for pg in p]
            o = tile_row(b * 2 * T + T + j,
                         lambda g, v: jnp.dot(p16[g], v, preferred_element_type=F32))
            return [l[g] + p[g] for g in groups], [acc[g] + o[g] for g in groups]

        zeros = [jnp.zeros((Q_ROWS, LANES), F32) for _ in groups]
        l, acc = lax.fori_loop(0, T, values, (zeros, zeros))
        for g in groups:
            o_scr[rows[g], :] = acc[g] / jnp.sum(l[g], axis=-1, keepdims=True)
        return carry

    lax.fori_loop(0, B, attend, 0)

    def o_chunk(i, acc):
        o = o_scr[_block(i, B), :].astype(BF16)
        return acc + lax.dot_general(o, columns(wo_buf, i), NT, preferred_element_type=F32)

    t = t_wg + U
    attn = stream.run(t, t + 2 * n_q, [(t, n_q, 2, o_chunk)], jnp.zeros((B, D), F32))
    x = x + mod(2) * attn
    h = _layernorm(x) * (1.0 + mod(4)) + mod(3)
    h16 = h.astype(BF16)

    def gate_chunk(f, carry):
        g_scr[f] = _silu(jnp.dot(h16, columns(wg_buf, f), preferred_element_type=F32))
        return carry

    stream.run(t + 2 * n_q, t_wd, [(t_wu, n_f, 2, gate_chunk)])

    small[2].wait()
    w_r = wr_buf[...].astype(F32).reshape(1, D)
    routed = jax.nn.sigmoid(jnp.sum(h16.astype(F32) * w_r, axis=-1, keepdims=True))
    tail_scr[0] = x + mod(5) * (h + h * 0.0)
    tail_scr[1] = mod(5) * routed

    def up(f):
        return (g_scr[f] * jnp.dot(h16, columns(wu_buf, f), preferred_element_type=F32)).astype(BF16)

    def down(a, f):
        return lax.dot_general(a, wd_buf[f], NT, preferred_element_type=F32)

    def down_step(f, carry):
        y, a = carry
        for u in range(2):
            stream.advance(t_wd + u, 2, f, n_f - 1)
        return y + down(a, f), up(f + 1)

    y, a = lax.fori_loop(0, n_f - 1, down_step, (jnp.zeros((B, D), F32), up(0)))
    for u in range(2):
        stream.advance(t_wd + 2 * (n_f - 1) + u)
    y = y + down(a, n_f - 1)
    out_ref[...] = (tail_scr[0] + tail_scr[1] * y).astype(out_ref.dtype)


@jax.jit
def pallas_adaLN_cond__sliding_block_cached__moe_arch_mod__decode_kernel(
    A_x: jax.Array,
    A_k_cache: jax.Array,
    A_v_cache: jax.Array,
    A_wq: jax.Array,
    A_wo: jax.Array,
    B_x: jax.Array,
    B_w_r: jax.Array,
    B_w_gate: jax.Array,
    B_w_up: jax.Array,
    B_w_down: jax.Array,
    c: jax.Array,
    w_mod: jax.Array,
):
    del B_x
    B, Sq, D = A_x.shape
    _, H, S, Dh = A_k_cache.shape
    Hq = A_wq.shape[1] // Dh
    F = B_w_gate.shape[1]
    W = min(4096, max(256, S // 4))
    assert Sq == 1 and Dh == LANES and Hq == 2 * H and D % (16 * BANDS) == 0

    def in_bands(w):
        return w.reshape(BANDS, D // BANDS, w.shape[1])

    def resident(n):
        return pltpu.VMEM((BANDS, D // BANDS, n), BF16)

    out = pl.pallas_call(
        _kernel,
        out_shape=jax.ShapeDtypeStruct((B, D), A_x.dtype),
        in_specs=[pl.BlockSpec(memory_space=pltpu.HBM)] * 11,
        out_specs=pl.BlockSpec(memory_space=pltpu.VMEM),
        scratch_shapes=[
            pltpu.VMEM((B, D), BF16),
            pltpu.VMEM((B, D), BF16),
            pltpu.VMEM((D,), BF16),
            pltpu.VMEM((KV_SLOTS, H, LANES, Dh), BF16),
            resident(w_mod.shape[1]),
            resident(Hq * Dh),
            resident(Hq * Dh),
            resident(F),
            resident(F),
            pltpu.VMEM((F // LANES, D, LANES), BF16),
            pltpu.VMEM((B, w_mod.shape[1]), F32),
            pltpu.VMEM((Hq * B, Dh), F32),
            pltpu.VMEM((W // LANES, Hq // Q_ROWS, Q_ROWS, LANES), F32),
            pltpu.VMEM((Hq * B, Dh), F32),
            pltpu.VMEM((F // LANES, B, LANES), F32),
            pltpu.VMEM((2, B, D), F32),
            pltpu.SemaphoreType.DMA((DEPTH,)),
            pltpu.SemaphoreType.DMA((3,)),
        ],
        compiler_params=pltpu.CompilerParams(
            vmem_limit_bytes=64 * 1024 * 1024,
            disable_bounds_checks=True,
            disable_semaphore_checks=True,
        ),
    )(
        A_x.reshape(B, D), A_k_cache, A_v_cache, in_bands(A_wq), in_bands(A_wo.T), B_w_r,
        in_bands(B_w_gate), in_bands(B_w_up), B_w_down.T, c, in_bands(w_mod),
    )
    return out.reshape(B, Sq, D)
```

```python
import math

import jax
import jax.numpy as jnp
from jax import lax
from jax.experimental import pallas as pl
from jax.experimental.pallas import tpu as pltpu

F32 = jnp.float32
BF16 = jnp.bfloat16
LANES = 128
NT = (((1,), (1,)), ((), ()))

DEPTH = 16
HEADS = 4
KEYS = 64
KV_SLOTS = 4
BANDS = 9
Q_ROWS = 16


def _div(i, n, limit):
    if isinstance(i, int):
        return i // n
    if n & (n - 1) == 0:
        return lax.shift_right_logical(i, jnp.int32(n.bit_length() - 1))
    magic = (1 << 16) // n + 1
    assert all((k * magic) >> 16 == k // n for k in range(limit))
    return lax.shift_right_logical(i * magic, jnp.int32(16))


def _mod(i, n):
    assert n & (n - 1) == 0
    return i % n if isinstance(i, int) else i & (n - 1)


def _block(i, n, base=0, align=None):
    start = base + i * n
    return pl.ds(start if isinstance(start, int) else pl.multiple_of(start, align or n), n)


def _runs(total, urgent):
    runs, lo = [], 0
    for first, count in urgent:
        runs += [(lo, first - lo, 1), (first, count, 0)]
        lo = first + count
    return [run for run in runs + [(lo, total - lo, 1)] if run[1]]


def _layernorm(x, eps=1e-5):
    d = x - jnp.mean(x, axis=-1, keepdims=True)
    return d / jnp.sqrt(jnp.mean(d * d, axis=-1, keepdims=True) + eps)


def _silu(x):
    return x * jax.nn.sigmoid(x)


def _pick(parts, owner):
    bit = 1
    while len(parts) > 1:
        even = (owner & bit) == 0
        parts = [jnp.where(even, a, b) for a, b in zip(parts[0::2], parts[1::2])]
        bit *= 2
    return parts[0]


class _Stream:
    def __init__(self, phases, sems):
        self.phases, self.sems = phases, sems
        self.bases = [0]
        for phase in phases:
            self.bases.append(self.bases[-1] + phase[0])

    def _each(self, t0, stride, it, n_it, act):
        sem = self.sems.at[_mod(t0 + stride * it, DEPTH)]
        for phase, first, end in zip(self.phases, self.bases, self.bases[1:]):
            last = t0 + stride * (n_it - 1)
            if last < first or t0 >= end:
                continue
            group = phase[1]
            assert n_it == 1 or stride % group == 0
            assert t0 >= first or last < end
            run = lambda: act(phase, (t0 - first) // group + stride // group * it, (t0 - first) % group, sem)
            if t0 < first:
                pl.when(t0 + stride * it >= first)(run)
            elif last >= end:
                pl.when(t0 + stride * it < end)(run)
            else:
                run()

    def start(self, t0, stride=1, it=0, n_it=1):
        self._each(t0, stride, it, n_it, lambda phase, i, u, sem: phase[2](i, u, sem))

    def advance(self, t0, stride=1, it=0, n_it=1):
        def wait(phase, i, u, sem):
            target = phase[3](i, u)
            pltpu.make_async_copy(target, target, sem).wait()

        self._each(t0, stride, it, n_it, wait)
        self.start(t0 + DEPTH, stride, it, n_it)

    def run(self, t0, t1, work=(), carry=0):
        cuts = {t0, t1, *self.bases, *(base - DEPTH for base in self.bases)}
        for first, n, every, _ in work:
            assert t0 <= first and first + n * every <= t1
            cuts |= {first, first + n * every}
        cuts = sorted(t for t in cuts if t0 <= t <= t1)
        for lo, hi in zip(cuts, cuts[1:]):
            jobs = [job for job in work if job[0] <= lo < job[0] + job[1] * job[2]]
            unroll = math.lcm(*(job[2] for job in jobs), *(
                phase[1] for phase, first, end in zip(self.phases, self.bases, self.bases[1:])
                if first <= lo < end or first <= lo + DEPTH < end))

            def step(t, it, n_it, carry):
                self.advance(t, unroll, it, n_it)
                for first, _, every, fn in jobs:
                    if (t - first) % every == every - 1:
                        carry = fn((t - first) // every + unroll // every * it, carry)
                return carry

            n_it = (hi - lo) // unroll
            if n_it > 1:
                def body(it, carry):
                    for u in range(unroll):
                        carry = step(lo + u, it, n_it, carry)
                    return carry

                carry = lax.fori_loop(0, n_it, body, carry)
                lo += n_it * unroll
            for t in range(lo, hi):
                carry = step(t, 0, 1, carry)
        return carry


def _kernel(x_hbm, k_hbm, v_hbm, wq_hbm, wo_hbm, wr_hbm, wg_hbm, wu_hbm, wd_hbm, c_hbm, wm_hbm,
            out_ref,
            x_buf, c_buf, wr_buf, kv_buf, wm_buf, wq_buf, wo_buf, wg_buf, wu_buf, wd_buf,
            mod_scr, q_scr, s_scr, o_scr, g_scr, tail_scr, sems, small_sems):
    B, D = x_buf.shape
    _, H, S, Dh = k_hbm.shape
    W = min(4096, max(256, S // 4))
    T = W // LANES
    U = H // HEADS * LANES // KEYS
    n_rows = B * 2 * T
    n_mod, n_q, n_f = (buf.shape[2] // LANES for buf in (wm_buf, wq_buf, wg_buf))
    n_mod1 = pl.cdiv(2 * D, LANES)
    assert DEPTH // U + 2 <= KV_SLOTS

    def banded(hbm, buf, chunk0, chunks, cols):
        n_cols = chunks * LANES // cols
        assert n_cols * cols == chunks * LANES
        steps = buf.shape[1] // 8 * n_cols

        def where(i):
            r = _div(i, n_cols, steps)
            return _block(r, 8), _block(i - r * n_cols, cols, chunk0 * LANES, LANES)

        def start(i, u, sem):
            for band, count, priority in _runs(BANDS, [(BANDS - 1, 1)]):
                at = (pl.ds(band, count), *where(i))
                pltpu.make_async_copy(hbm.at[at], buf.at[at], sem).start(priority=priority)

        return steps, 1, start, lambda i, u: buf.at[(slice(None), *where(i))]

    def kv_target(n, u, first=0, count=HEADS):
        head = u % (H // HEADS) * HEADS + first
        return kv_buf.at[_mod(n, KV_SLOTS), pl.ds(head, count), _block(u // (H // HEADS), KEYS)]

    def kv_start(n, u, sem):
        keys = _block(_mod(n, T) * (LANES // KEYS) + u // (H // HEADS), KEYS, S - W)

        def start_from(hbm):
            for first, count, priority in _runs(HEADS, [(HEADS - 1, 1)]):
                heads = pl.ds(u % (H // HEADS) * HEADS + first, count)
                pltpu.make_async_copy(hbm.at[_div(n, 2 * T, n_rows), heads, keys],
                                      kv_target(n, u, first, count), sem).start(priority=priority)

        is_value = _mod(_div(n, T, n_rows), 2)
        if isinstance(is_value, int):
            start_from(v_hbm if is_value else k_hbm)
        else:
            pl.when(is_value == 0)(lambda: start_from(k_hbm))
            pl.when(is_value == 1)(lambda: start_from(v_hbm))

    def down_start(f, u, sem):
        for row, count, priority in _runs(D // 2, [(D // 2 - 16, 16)]):
            rows = pl.ds(u * (D // 2) + row, count)
            pltpu.make_async_copy(
                wd_hbm.at[rows, _block(f, LANES)], wd_buf.at[f, rows], sem).start(priority=priority)

    stream = _Stream([
        banded(wm_hbm, wm_buf, 0, n_mod1, 384),
        banded(wq_hbm, wq_buf, 0, n_q, 512),
        banded(wm_hbm, wm_buf, n_mod1, n_mod - n_mod1, 384),
        banded(wo_hbm, wo_buf, 0, n_q, 512),
        (n_rows * U, U, kv_start, kv_target),
        banded(wg_hbm, wg_buf, 0, n_f, 512),
        banded(wu_hbm, wu_buf, 0, n_f, 512),
        (2 * n_f, 2, down_start, lambda f, u: wd_buf.at[f, _block(u, D // 2)]),
    ], sems)
    t_wq, t_wm2, t_wo, t_kv, t_wg, t_wu, t_wd = stream.bases[1:-1]

    def columns(buf, i, n=1):
        return buf[:, :, _block(i, n * LANES)].reshape(D, n * LANES)

    small = [pltpu.make_async_copy(src, dst, small_sems.at[n])
             for n, (src, dst) in enumerate(((c_hbm, c_buf), (x_hbm, x_buf), (wr_hbm, wr_buf)))]
    stream.start(0)
    for copy in small:
        copy.start()
    for t in range(1, DEPTH):
        stream.start(t)

    small[0].wait()
    cond = _silu(c_buf[...].astype(F32)).astype(BF16)

    def mod_chunk(first):
        def fn(i, carry):
            mod_scr[:, _block(first + i, LANES)] = jnp.dot(
                cond, columns(wm_buf, first + i), preferred_element_type=F32)
            return carry
        return fn

    def mod(i):
        return mod_scr[:, i * D:(i + 1) * D]

    t = t_wq + 2 * n_mod1
    stream.run(0, t, [(t_wq, n_mod1, 2, mod_chunk(0))])
    small[1].wait()
    x = x_buf[...].astype(F32)
    h = (_layernorm(x) * (1.0 + mod(1)) + mod(0)).astype(BF16)

    def q_chunk(i, carry):
        q = jnp.dot(h, columns(wq_buf, i, 2), preferred_element_type=F32)
        for n in range(2):
            q_scr[_block(2 * i + n, B), :] = q[:, n * LANES:(n + 1) * LANES]
        return carry

    stream.run(t, t_kv + U, [(t_wm2, n_q // 2, 3, q_chunk), (t_wo, n_mod - n_mod1, 2, mod_chunk(n_mod1))])

    G = Q_ROWS // 2
    groups = range(H // G)
    owner = lax.broadcasted_iota(jnp.int32, (Q_ROWS, LANES), 0) // 2
    scale = Dh ** -0.5

    def tile_row(n, product):
        parts = []
        for u in range(U):
            stream.advance(t_kv + U + u, U, n, n_rows)
            if u % 2 == 0:
                parts += [product(head // G, kv_buf[_mod(n, KV_SLOTS), head])
                          for head in range(u * H // U, (u + 2) * H // U)]
        return [_pick(parts[g * G:(g + 1) * G], owner) for g in groups]

    def attend(b, carry):
        rows = [pl.ds(g * Q_ROWS * B + b, Q_ROWS, stride=B) for g in groups]
        q = [q_scr[r, :].astype(BF16) for r in rows]

        def scores(j, m):
            s = tile_row(b * 2 * T + j,
                         lambda g, k: lax.dot_general(q[g], k, NT, preferred_element_type=F32))
            for g in groups:
                s_scr[j, g] = s[g]
            return [jnp.maximum(m[g], s[g]) for g in groups]

        m = lax.fori_loop(0, T, scores, [jnp.full((Q_ROWS, LANES), -jnp.inf, F32) for _ in groups])
        m = [jnp.broadcast_to(jnp.max(mg, axis=-1, keepdims=True), mg.shape) for mg in m]

        def values(j, carry):
            l, acc = carry
            p = [jnp.exp((s_scr[j, g] - m[g]) * scale) for g in groups]
            p16 = [pg.astype(BF16) for pg in p]
            o = tile_row(b * 2 * T + T + j,
                         lambda g, v: jnp.dot(p16[g], v, preferred_element_type=F32))
            return [l[g] + p[g] for g in groups], [acc[g] + o[g] for g in groups]

        zeros = [jnp.zeros((Q_ROWS, LANES), F32) for _ in groups]
        l, acc = lax.fori_loop(0, T, values, (zeros, zeros))
        for g in groups:
            o_scr[rows[g], :] = acc[g] / jnp.sum(l[g], axis=-1, keepdims=True)
        return carry

    lax.fori_loop(0, B, attend, 0)

    def o_chunk(i, acc):
        o = o_scr[_block(i, B), :].astype(BF16)
        return acc + lax.dot_general(o, columns(wo_buf, i), NT, preferred_element_type=F32)

    t = t_wg + U
    attn = stream.run(t, t + 2 * n_q, [(t, n_q, 2, o_chunk)], jnp.zeros((B, D), F32))
    x = x + mod(2) * attn
    h = _layernorm(x) * (1.0 + mod(4)) + mod(3)
    h16 = h.astype(BF16)

    def gate_chunk(f, carry):
        g_scr[f] = _silu(jnp.dot(h16, columns(wg_buf, f), preferred_element_type=F32))
        return carry

    stream.run(t + 2 * n_q, t_wd, [(t_wu, n_f, 2, gate_chunk)])

    small[2].wait()
    w_r = wr_buf[...].astype(F32).reshape(1, D)
    routed = jax.nn.sigmoid(jnp.sum(h16.astype(F32) * w_r, axis=-1, keepdims=True))
    tail_scr[0] = x + mod(5) * (h + h * 0.0)
    tail_scr[1] = mod(5) * routed

    def up(f):
        return (g_scr[f] * jnp.dot(h16, columns(wu_buf, f), preferred_element_type=F32)).astype(BF16)

    def down(a, f):
        return lax.dot_general(a, wd_buf[f], NT, preferred_element_type=F32)

    def down_step(f, carry):
        y, a = carry
        for u in range(2):
            stream.advance(t_wd + u, 2, f, n_f - 1)
        return y + down(a, f), up(f + 1)

    y, a = lax.fori_loop(0, n_f - 1, down_step, (jnp.zeros((B, D), F32), up(0)))
    for u in range(2):
        stream.advance(t_wd + 2 * (n_f - 1) + u)
    y = y + down(a, n_f - 1)
    out_ref[...] = (tail_scr[0] + tail_scr[1] * y).astype(out_ref.dtype)


@jax.jit
def pallas_adaLN_cond__sliding_block_cached__moe_arch_mod__decode_kernel(
    A_x: jax.Array,
    A_k_cache: jax.Array,
    A_v_cache: jax.Array,
    A_wq: jax.Array,
    A_wo: jax.Array,
    B_x: jax.Array,
    B_w_r: jax.Array,
    B_w_gate: jax.Array,
    B_w_up: jax.Array,
    B_w_down: jax.Array,
    c: jax.Array,
    w_mod: jax.Array,
):
    del B_x
    B, Sq, D = A_x.shape
    _, H, S, Dh = A_k_cache.shape
    Hq = A_wq.shape[1] // Dh
    F = B_w_gate.shape[1]
    W = min(4096, max(256, S // 4))
    assert Sq == 1 and Dh == LANES and Hq == 2 * H and D % (16 * BANDS) == 0

    def in_bands(w):
        return w.reshape(BANDS, D // BANDS, w.shape[1])

    def resident(n):
        return pltpu.VMEM((BANDS, D // BANDS, n), BF16)

    out = pl.pallas_call(
        _kernel,
        out_shape=jax.ShapeDtypeStruct((B, D), A_x.dtype),
        in_specs=[pl.BlockSpec(memory_space=pltpu.HBM)] * 11,
        out_specs=pl.BlockSpec(memory_space=pltpu.VMEM),
        scratch_shapes=[
            pltpu.VMEM((B, D), BF16),
            pltpu.VMEM((B, D), BF16),
            pltpu.VMEM((D,), BF16),
            pltpu.VMEM((KV_SLOTS, H, LANES, Dh), BF16),
            resident(w_mod.shape[1]),
            resident(Hq * Dh),
            resident(Hq * Dh),
            resident(F),
            resident(F),
            pltpu.VMEM((F // LANES, D, LANES), BF16),
            pltpu.VMEM((B, w_mod.shape[1]), F32),
            pltpu.VMEM((Hq * B, Dh), F32),
            pltpu.VMEM((W // LANES, Hq // Q_ROWS, Q_ROWS, LANES), F32),
            pltpu.VMEM((Hq * B, Dh), F32),
            pltpu.VMEM((F // LANES, B, LANES), F32),
            pltpu.VMEM((2, B, D), F32),
            pltpu.SemaphoreType.DMA((DEPTH,)),
            pltpu.SemaphoreType.DMA((3,)),
        ],
        compiler_params=pltpu.CompilerParams(
            vmem_limit_bytes=64 * 1024 * 1024,
            disable_bounds_checks=True,
            disable_semaphore_checks=True,
        ),
    )(
        A_x.reshape(B, D), A_k_cache, A_v_cache, in_bands(A_wq), in_bands(A_wo.T), B_w_r,
        in_bands(B_w_gate), in_bands(B_w_up), B_w_down.T, c, in_bands(w_mod),
    )
    return out.reshape(B, Sq, D)
```

```python
import math

import jax
import jax.numpy as jnp
from jax import lax
from jax.experimental import pallas as pl
from jax.experimental.pallas import tpu as pltpu

F32 = jnp.float32
BF16 = jnp.bfloat16
LANES = 128
NT = (((1,), (1,)), ((), ()))

DEPTH = 16
HEADS = 4
KEYS = 64
KV_SLOTS = 4
BANDS = 9
Q_ROWS = 16


def _div(i, n, limit):
    if isinstance(i, int):
        return i // n
    if n & (n - 1) == 0:
        return lax.shift_right_logical(i, jnp.int32(n.bit_length() - 1))
    magic = (1 << 16) // n + 1
    assert all((k * magic) >> 16 == k // n for k in range(limit))
    return lax.shift_right_logical(i * magic, jnp.int32(16))


def _mod(i, n):
    assert n & (n - 1) == 0
    return i % n if isinstance(i, int) else i & (n - 1)


def _block(i, n, base=0, align=None):
    start = base + i * n
    return pl.ds(start if isinstance(start, int) else pl.multiple_of(start, align or n), n)


def _runs(total, urgent):
    runs, lo = [], 0
    for first, count in urgent:
        runs += [(lo, first - lo, 1), (first, count, 0)]
        lo = first + count
    return [run for run in runs + [(lo, total - lo, 1)] if run[1]]


def _layernorm(x, eps=1e-5):
    d = x - jnp.mean(x, axis=-1, keepdims=True)
    return d / jnp.sqrt(jnp.mean(d * d, axis=-1, keepdims=True) + eps)


def _silu(x):
    return x * jax.nn.sigmoid(x)


def _pick(parts, owner):
    bit = 1
    while len(parts) > 1:
        even = (owner & bit) == 0
        parts = [jnp.where(even, a, b) for a, b in zip(parts[0::2], parts[1::2])]
        bit *= 2
    return parts[0]


class _Stream:
    def __init__(self, phases, sems):
        self.phases, self.sems = phases, sems
        self.bases = [0]
        for phase in phases:
            self.bases.append(self.bases[-1] + phase[0])

    def _each(self, t0, stride, it, n_it, act):
        sem = self.sems.at[_mod(t0 + stride * it, DEPTH)]
        for phase, first, end in zip(self.phases, self.bases, self.bases[1:]):
            last = t0 + stride * (n_it - 1)
            if last < first or t0 >= end:
                continue
            group = phase[1]
            assert n_it == 1 or stride % group == 0
            assert t0 >= first or last < end
            run = lambda: act(phase, (t0 - first) // group + stride // group * it, (t0 - first) % group, sem)
            if t0 < first:
                pl.when(t0 + stride * it >= first)(run)
            elif last >= end:
                pl.when(t0 + stride * it < end)(run)
            else:
                run()

    def start(self, t0, stride=1, it=0, n_it=1):
        self._each(t0, stride, it, n_it, lambda phase, i, u, sem: phase[2](i, u, sem))

    def advance(self, t0, stride=1, it=0, n_it=1):
        def wait(phase, i, u, sem):
            target = phase[3](i, u)
            pltpu.make_async_copy(target, target, sem).wait()

        self._each(t0, stride, it, n_it, wait)
        self.start(t0 + DEPTH, stride, it, n_it)

    def run(self, t0, t1, work=(), carry=0):
        cuts = {t0, t1, *self.bases, *(base - DEPTH for base in self.bases)}
        for first, n, every, _ in work:
            assert t0 <= first and first + n * every <= t1
            cuts |= {first, first + n * every}
        cuts = sorted(t for t in cuts if t0 <= t <= t1)
        for lo, hi in zip(cuts, cuts[1:]):
            jobs = [job for job in work if job[0] <= lo < job[0] + job[1] * job[2]]
            unroll = math.lcm(*(job[2] for job in jobs), *(
                phase[1] for phase, first, end in zip(self.phases, self.bases, self.bases[1:])
                if first <= lo < end or first <= lo + DEPTH < end))

            def step(t, it, n_it, carry):
                self.advance(t, unroll, it, n_it)
                for first, _, every, fn in jobs:
                    if (t - first) % every == every - 1:
                        carry = fn((t - first) // every + unroll // every * it, carry)
                return carry

            n_it = (hi - lo) // unroll
            if n_it > 1:
                def body(it, carry):
                    for u in range(unroll):
                        carry = step(lo + u, it, n_it, carry)
                    return carry

                carry = lax.fori_loop(0, n_it, body, carry)
                lo += n_it * unroll
            for t in range(lo, hi):
                carry = step(t, 0, 1, carry)
        return carry


def _kernel(x_hbm, k_hbm, v_hbm, wq_hbm, wo_hbm, wr_hbm, wg_hbm, wu_hbm, wd_hbm, c_hbm, wm_hbm,
            out_ref,
            x_buf, c_buf, wr_buf, kv_buf, wm_buf, wq_buf, wo_buf, wg_buf, wu_buf, wd_buf,
            mod_scr, q_scr, s_scr, o_scr, g_scr, tail_scr, sems, small_sems):
    B, D = x_buf.shape
    _, H, S, Dh = k_hbm.shape
    W = min(4096, max(256, S // 4))
    T = W // LANES
    U = H // HEADS * LANES // KEYS
    n_rows = B * 2 * T
    n_mod, n_q, n_f = (buf.shape[2] // LANES for buf in (wm_buf, wq_buf, wg_buf))
    n_mod1 = pl.cdiv(2 * D, LANES)
    assert DEPTH // U + 2 <= KV_SLOTS

    def banded(hbm, buf, chunk0, chunks, cols):
        n_cols = chunks * LANES // cols
        assert n_cols * cols == chunks * LANES
        steps = buf.shape[1] // 8 * n_cols

        def where(i):
            r = _div(i, n_cols, steps)
            return _block(r, 8), _block(i - r * n_cols, cols, chunk0 * LANES, LANES)

        def start(i, u, sem):
            for band, count, priority in _runs(BANDS, [(BANDS - 1, 1)]):
                at = (pl.ds(band, count), *where(i))
                pltpu.make_async_copy(hbm.at[at], buf.at[at], sem).start(priority=priority)

        return steps, 1, start, lambda i, u: buf.at[(slice(None), *where(i))]

    def kv_target(n, u, first=0, count=HEADS):
        head = u % (H // HEADS) * HEADS + first
        return kv_buf.at[_mod(n, KV_SLOTS), pl.ds(head, count), _block(u // (H // HEADS), KEYS)]

    def kv_start(n, u, sem):
        keys = _block(_mod(n, T) * (LANES // KEYS) + u // (H // HEADS), KEYS, S - W)

        def start_from(hbm):
            for first, count, priority in _runs(HEADS, [(HEADS - 1, 1)]):
                heads = pl.ds(u % (H // HEADS) * HEADS + first, count)
                pltpu.make_async_copy(hbm.at[_div(n, 2 * T, n_rows), heads, keys],
                                      kv_target(n, u, first, count), sem).start(priority=priority)

        is_value = _mod(_div(n, T, n_rows), 2)
        if isinstance(is_value, int):
            start_from(v_hbm if is_value else k_hbm)
        else:
            pl.when(is_value == 0)(lambda: start_from(k_hbm))
            pl.when(is_value == 1)(lambda: start_from(v_hbm))

    def down_start(f, u, sem):
        for row, count, priority in _runs(D // 2, [(D // 2 - 16, 16)]):
            rows = pl.ds(u * (D // 2) + row, count)
            pltpu.make_async_copy(
                wd_hbm.at[rows, _block(f, LANES)], wd_buf.at[f, rows], sem).start(priority=priority)

    stream = _Stream([
        banded(wm_hbm, wm_buf, 0, n_mod1, 384),
        banded(wq_hbm, wq_buf, 0, n_q, 512),
        banded(wm_hbm, wm_buf, n_mod1, n_mod - n_mod1, 384),
        banded(wo_hbm, wo_buf, 0, n_q, 512),
        (n_rows * U, U, kv_start, kv_target),
        banded(wg_hbm, wg_buf, 0, n_f, 512),
        banded(wu_hbm, wu_buf, 0, n_f, 512),
        (2 * n_f, 2, down_start, lambda f, u: wd_buf.at[f, _block(u, D // 2)]),
    ], sems)
    t_wq, t_wm2, t_wo, t_kv, t_wg, t_wu, t_wd = stream.bases[1:-1]

    def columns(buf, i, n=1):
        return buf[:, :, _block(i, n * LANES)].reshape(D, n * LANES)

    small = [pltpu.make_async_copy(src, dst, small_sems.at[n])
             for n, (src, dst) in enumerate(((c_hbm, c_buf), (x_hbm, x_buf), (wr_hbm, wr_buf)))]
    stream.start(0)
    for copy in small:
        copy.start()
    for t in range(1, DEPTH):
        stream.start(t)

    small[0].wait()
    cond = _silu(c_buf[...].astype(F32)).astype(BF16)

    def mod_chunk(first):
        def fn(i, carry):
            mod_scr[:, _block(first + i, LANES)] = jnp.dot(
                cond, columns(wm_buf, first + i), preferred_element_type=F32)
            return carry
        return fn

    def mod(i):
        return mod_scr[:, i * D:(i + 1) * D]

    t = t_wq + 2 * n_mod1
    stream.run(0, t, [(t_wq, n_mod1, 2, mod_chunk(0))])
    small[1].wait()
    x = x_buf[...].astype(F32)
    h = (_layernorm(x) * (1.0 + mod(1)) + mod(0)).astype(BF16)

    def q_chunk(i, carry):
        q = jnp.dot(h, columns(wq_buf, i, 2), preferred_element_type=F32)
        for n in range(2):
            q_scr[_block(2 * i + n, B), :] = q[:, n * LANES:(n + 1) * LANES]
        return carry

    stream.run(t, t_kv + U, [(t_wm2, n_q // 2, 3, q_chunk), (t_wo, n_mod - n_mod1, 2, mod_chunk(n_mod1))])

    G = Q_ROWS // 2
    groups = range(H // G)
    owner = lax.broadcasted_iota(jnp.int32, (Q_ROWS, LANES), 0) // 2
    scale = Dh ** -0.5

    def tile_row(n, product):
        parts = []
        for u in range(U):
            stream.advance(t_kv + U + u, U, n, n_rows)
            if u % 2 == 0:
                parts += [product(head // G, kv_buf[_mod(n, KV_SLOTS), head])
                          for head in range(u * H // U, (u + 2) * H // U)]
        return [_pick(parts[g * G:(g + 1) * G], owner) for g in groups]

    def attend(b, carry):
        rows = [pl.ds(g * Q_ROWS * B + b, Q_ROWS, stride=B) for g in groups]
        q = [q_scr[r, :].astype(BF16) for r in rows]

        def scores(j, m):
            s = tile_row(b * 2 * T + j,
                         lambda g, k: lax.dot_general(q[g], k, NT, preferred_element_type=F32))
            for g in groups:
                s_scr[j, g] = s[g]
            return [jnp.maximum(m[g], s[g]) for g in groups]

        m = lax.fori_loop(0, T, scores, [jnp.full((Q_ROWS, LANES), -jnp.inf, F32) for _ in groups])
        m = [jnp.broadcast_to(jnp.max(mg, axis=-1, keepdims=True), mg.shape) for mg in m]

        def values(j, carry):
            l, acc = carry
            p = [jnp.exp((s_scr[j, g] - m[g]) * scale) for g in groups]
            p16 = [pg.astype(BF16) for pg in p]
            o = tile_row(b * 2 * T + T + j,
                         lambda g, v: jnp.dot(p16[g], v, preferred_element_type=F32))
            return [l[g] + p[g] for g in groups], [acc[g] + o[g] for g in groups]

        zeros = [jnp.zeros((Q_ROWS, LANES), F32) for _ in groups]
        l, acc = lax.fori_loop(0, T, values, (zeros, zeros))
        for g in groups:
            o_scr[rows[g], :] = acc[g] / jnp.sum(l[g], axis=-1, keepdims=True)
        return carry

    lax.fori_loop(0, B, attend, 0)

    def o_chunk(i, acc):
        o = o_scr[_block(i, B), :].astype(BF16)
        return acc + lax.dot_general(o, columns(wo_buf, i), NT, preferred_element_type=F32)

    t = t_wg + U
    attn = stream.run(t, t + 2 * n_q, [(t, n_q, 2, o_chunk)], jnp.zeros((B, D), F32))
    x = x + mod(2) * attn
    h = _layernorm(x) * (1.0 + mod(4)) + mod(3)
    h16 = h.astype(BF16)

    def gate_chunk(f, carry):
        g_scr[f] = _silu(jnp.dot(h16, columns(wg_buf, f), preferred_element_type=F32))
        return carry

    stream.run(t + 2 * n_q, t_wd, [(t_wu, n_f, 2, gate_chunk)])

    small[2].wait()
    w_r = wr_buf[...].astype(F32).reshape(1, D)
    routed = jax.nn.sigmoid(jnp.sum(h16.astype(F32) * w_r, axis=-1, keepdims=True))
    tail_scr[0] = x + mod(5) * (h + h * 0.0)
    tail_scr[1] = mod(5) * routed

    n_up = 3

    def up(i):
        u = jnp.dot(h16, columns(wu_buf, i, n_up), preferred_element_type=F32)
        for n in range(n_up):
            g_scr[n_up * i + n] = g_scr[n_up * i + n] * u[:, n * LANES:(n + 1) * LANES]

    def down(f, y):
        return y + lax.dot_general(g_scr[f].astype(BF16), wd_buf[f], NT, preferred_element_type=F32)

    def down_and_up(f, y):
        y = down(f, y)
        up(f + 1)
        return y

    up(0)
    n_early = n_f // n_up - 1
    y = stream.run(t_wd, stream.bases[-1], [
        (t_wd, n_early, 2, down_and_up),
        (t_wd + 2 * n_early, n_f - n_early, 2, lambda i, y: down(n_early + i, y)),
    ], jnp.zeros((B, D), F32))
    out_ref[...] = (tail_scr[0] + tail_scr[1] * y).astype(out_ref.dtype)


@jax.jit
def pallas_adaLN_cond__sliding_block_cached__moe_arch_mod__decode_kernel(
    A_x: jax.Array,
    A_k_cache: jax.Array,
    A_v_cache: jax.Array,
    A_wq: jax.Array,
    A_wo: jax.Array,
    B_x: jax.Array,
    B_w_r: jax.Array,
    B_w_gate: jax.Array,
    B_w_up: jax.Array,
    B_w_down: jax.Array,
    c: jax.Array,
    w_mod: jax.Array,
):
    del B_x
    B, Sq, D = A_x.shape
    _, H, S, Dh = A_k_cache.shape
    Hq = A_wq.shape[1] // Dh
    F = B_w_gate.shape[1]
    W = min(4096, max(256, S // 4))
    assert Sq == 1 and Dh == LANES and Hq == 2 * H and D % (16 * BANDS) == 0 and F % (3 * LANES) == 0

    def in_bands(w):
        return w.reshape(BANDS, D // BANDS, w.shape[1])

    def resident(n):
        return pltpu.VMEM((BANDS, D // BANDS, n), BF16)

    out = pl.pallas_call(
        _kernel,
        out_shape=jax.ShapeDtypeStruct((B, D), A_x.dtype),
        in_specs=[pl.BlockSpec(memory_space=pltpu.HBM)] * 11,
        out_specs=pl.BlockSpec(memory_space=pltpu.VMEM),
        scratch_shapes=[
            pltpu.VMEM((B, D), BF16),
            pltpu.VMEM((B, D), BF16),
            pltpu.VMEM((D,), BF16),
            pltpu.VMEM((KV_SLOTS, H, LANES, Dh), BF16),
            resident(w_mod.shape[1]),
            resident(Hq * Dh),
            resident(Hq * Dh),
            resident(F),
            resident(F),
            pltpu.VMEM((F // LANES, D, LANES), BF16),
            pltpu.VMEM((B, w_mod.shape[1]), F32),
            pltpu.VMEM((Hq * B, Dh), F32),
            pltpu.VMEM((W // LANES, Hq // Q_ROWS, Q_ROWS, LANES), F32),
            pltpu.VMEM((Hq * B, Dh), F32),
            pltpu.VMEM((F // LANES, B, LANES), F32),
            pltpu.VMEM((2, B, D), F32),
            pltpu.SemaphoreType.DMA((DEPTH,)),
            pltpu.SemaphoreType.DMA((3,)),
        ],
        compiler_params=pltpu.CompilerParams(
            vmem_limit_bytes=64 * 1024 * 1024,
            disable_bounds_checks=True,
            disable_semaphore_checks=True,
        ),
    )(
        A_x.reshape(B, D), A_k_cache, A_v_cache, in_bands(A_wq), in_bands(A_wo.T), B_w_r,
        in_bands(B_w_gate), in_bands(B_w_up), B_w_down.T, c, in_bands(w_mod),
    )
    return out.reshape(B, Sq, D)
```
